```python
import os as _os
_os.environ.setdefault("JAX_PLATFORMS", "cpu")
import jax
import jax.numpy as jnp

def _softmax(x, axis=-1):
    return jax.nn.softmax(x, axis=axis)
def _gelu(x):
    return jax.nn.gelu(x, approximate=True)
def _silu(x):
    return jax.nn.silu(x)
def _sigmoid(x):
    return jax.nn.sigmoid(x)
def _layernorm(x, axis=-1, eps=1e-5):
    m = jnp.mean(x, axis=axis, keepdims=True)
    v = jnp.var(x, axis=axis, keepdims=True)
    return (x - m) / jnp.sqrt(v + eps)
def _scatter_add(tgt, idx, src, axis=0):
    return tgt.at[idx].add(src)
def _segment_sum(src, seg, n):
    return jax.ops.segment_sum(src, seg, n)
class _Rng:
    def __init__(self, key):
        self._k = key
    def _next(self):
        self._k, sub = jax.random.split(self._k)
        return sub
    def normal(self, shape):
        return jax.random.normal(self._next(), shape, dtype=jnp.bfloat16)
    def randint(self, lo, hi, shape):
        return jax.random.randint(self._next(), shape, lo, hi, dtype=jnp.int32)
    def uniform(self, shape, lo=0.0, hi=1.0):
        return jax.random.uniform(self._next(), shape, jnp.bfloat16, lo, hi)
    def permutation(self, n):
        return jax.random.permutation(self._next(), n)


kernel_name = 'gated_mix__sliding_local_dilated__moe_arch_mod__prompt'

def setup_inputs():
    _rng = _Rng(jax.random.key(int.from_bytes(__import__("os").urandom(4), "little")))
    _w = (lambda a: (lambda t: t.astype(jnp.bfloat16) if jnp.issubdtype(t.dtype, jnp.floating) else t)(jnp.asarray(a)))
    def _A_setup():
        B, S, D = 1, 2048, 640
        return {
            "x": _w((lambda *s: _rng.normal(s) * 0.05)(B, S, D)),
            "wqkv": _w((lambda *s: _rng.normal(s) * 0.8)(D, 3 * D)),
            "wo": _w((lambda *s: _rng.normal(s) * 0.05)(D, D)),
        }
    _A_in = _A_setup()

    def _B_setup():
        B, S, D, F, C = 1, 2048, 640, 1728, 1
        return {
            "x": _w((lambda *s: _rng.normal(s) * 0.05)(B, S, D)),
            "w_r": _w((lambda *s: _rng.normal(s) * 1.6)(D)),
            "w_gate": _w((lambda *s: _rng.normal(s) * 0.4)(D, F)),
            "w_up": _w((lambda *s: _rng.normal(s) * 0.4)(D, F)),
            "w_down": _w((lambda *s: _rng.normal(s) * 0.4)(F, D)),
        }
    _B_in = _B_setup()

    return {
        "A_x": _A_in["x"],
        "A_wqkv": _A_in["wqkv"],
        "A_wo": _A_in["wo"],
        "B_x": _B_in["x"],
        "B_w_r": _B_in["w_r"],
        "B_w_gate": _B_in["w_gate"],
        "B_w_up": _B_in["w_up"],
        "B_w_down": _B_in["w_down"],
        "gate_w": _w((lambda *s: _rng.normal(s) * 0.05)(640) * 16.0),
    }

def reference(A_x, A_wqkv, A_wo, B_x, B_w_r, B_w_gate, B_w_up, B_w_down, gate_w):
    def _A_ref(x, wqkv, wo):
        B, S, D = x.shape
        H = 32; Dh = D // H
        W, dil = 8, 2
        qkv = (lambda x, *d: x.transpose(*d))((x @ wqkv).reshape(B, S, 3, H, Dh), 2, 0, 3, 1, 4)
        q, k, v = qkv[0], qkv[1], qkv[2]
        scale = Dh ** -0.5
        pos = jnp.arange(S)
        off = jnp.arange(W) * dil
        idx = pos[:, None] - off[None, :]
        mask = idx >= 0
        idx_c = jnp.where(mask, idx, 0).reshape(-1)
        kg = k[:, :, idx_c, :].reshape(B, H, S, W, Dh)
        vg = v[:, :, idx_c, :].reshape(B, H, S, W, Dh)
        logits = jnp.einsum("bhsd,bhswd->bhsw", q, kg) * scale
        logits = jnp.where(mask[None, None, :, :], logits, -1e9)
        attn = _softmax(logits, axis=-1)
        o = jnp.einsum("bhsw,bhswd->bhsd", attn, vg)
        return (lambda x, *d: x.transpose(*d))(o, 0, 2, 1, 3).reshape(B, S, D) @ wo

    def _B_ref(x, w_r, w_gate, w_up, w_down):
        B, S, D = x.shape
        C = 1
        r = x @ w_r
        idx = jnp.argsort(-r, axis=-1)[:, :C]
        idx_e = jnp.repeat(idx.reshape(B, C, 1), D, axis=2)
        x_sel = jnp.take_along_axis(x, idx_e, axis=1)
        g = _silu(x_sel @ w_gate)
        u = x_sel @ w_up
        y = (g * u) @ w_down
        r_sel = _sigmoid(jnp.take_along_axis(r, idx, axis=1))
        y = y * r_sel.reshape(B, C, 1)
        b_off = (jnp.arange(B) * S).reshape(B, 1)
        flat_idx = (idx + b_off).reshape(B * C)
        zero = (x * 0.0).reshape(B * S, D)
        upd = _scatter_add(zero, flat_idx, y.reshape(B * C, D), axis=0)
        return x + upd.reshape(B, S, D)

    x = A_x
    g = _sigmoid((x * gate_w).sum(-1, keepdims=True))
    a = _A_ref(x, A_wqkv, A_wo)
    b = _B_ref(x, B_w_r, B_w_gate, B_w_up, B_w_down)
    return g * a + (1 - g) * b
```

```python
import functools, math
import jax
import jax.numpy as jnp
import jax.experimental.pallas as pl
import jax.experimental.pallas.tpu as pltpu

S, D, H, DH, WIN, DIL, F = 2048, 640, 32, 20, 8, 2, 1728
NL = D // 128
HALO = 16
f32, bf16 = jnp.float32, jnp.bfloat16
QSCALE = (DH ** -0.5) * math.log2(math.e)
NT = (((1,), (1,)), ((), ()))


def make(TM=256, RG=64, FFN_AT=3):
    NB = S // TM

    def kernel(x_hbm, wqkv_hbm, wo_hbm, wr_ref, wg_hbm, wu_hbm, wd_hbm, gw_ref, out_hbm,
               x_v, wqkv_v, wo_v, wg_v, wu_v, wd_v, out_v,
               t_ref, wp_ref, wop_ref, q_ref, k_ref, v_ref, o_ref, y_ref, idx_ref,
               sem_w, sem_x, sem_f, sem_o):
        def wcopy(p):
            return pltpu.make_async_copy(wqkv_hbm.at[:, p * D:(p + 1) * D], wqkv_v.at[:, p * D:(p + 1) * D], sem_w.at[p])
        def xcopy(i):
            return pltpu.make_async_copy(x_hbm.at[0, i * TM:(i + 1) * TM, :], x_v.at[i * TM:(i + 1) * TM, :], sem_x.at[i])
        def ocopy(i):
            return pltpu.make_async_copy(out_v.at[i * TM:(i + 1) * TM, :], out_hbm.at[0, i * TM:(i + 1) * TM, :], sem_o.at[i])
        wocopy = pltpu.make_async_copy(wo_hbm, wo_v, sem_w.at[3])
        fcopies = [pltpu.make_async_copy(a, b, sem_f.at[n]) for n, (a, b) in
                   enumerate(((wg_hbm, wg_v), (wu_hbm, wu_v), (wd_hbm, wd_v)))]

        wcopy(0).start(); xcopy(0).start(); wcopy(1).start()

        for j in range(NL):
            k_ref[j, 0:HALO, :] = jnp.zeros((HALO, 128), f32)
            v_ref[j, 0:HALO, :] = jnp.zeros((HALO, 128), f32)

        def prep_w(p):
            for kt in range(NL):
                w = wqkv_v[kt * 128:(kt + 1) * 128, p * D:(p + 1) * D]
                t_ref[p * NL + kt] = w.T.astype(f32)
                for d in range(DH):
                    wp_ref[p * D + d * H: p * D + (d + 1) * H, kt * 128:(kt + 1) * 128] = (
                        t_ref[p * NL + kt, pl.ds(d, H, stride=DH), :].astype(bf16))

        def prep_wo():
            for kt in range(NL):
                t_ref[3 * NL + kt] = wo_v[:, kt * 128:(kt + 1) * 128].astype(f32)
                for d in range(DH):
                    wop_ref[d * H:(d + 1) * H, kt * 128:(kt + 1) * 128] = (
                        t_ref[3 * NL + kt, pl.ds(d, H, stride=DH), :].astype(bf16))

        def qkv_part(i, p):
            xb = x_v[i * TM:(i + 1) * TM, :]
            r = jax.lax.dot_general(xb, wp_ref[p * D:(p + 1) * D, :], NT, preferred_element_type=f32)
            for j in range(NL):
                rj = r[:, j * 128:(j + 1) * 128]
                if p == 0:
                    q_ref[j, i * TM:(i + 1) * TM, :] = rj * QSCALE
                elif p == 1:
                    k_ref[j, HALO + i * TM:HALO + (i + 1) * TM, :] = rj
                else:
                    v_ref[j, HALO + i * TM:HALO + (i + 1) * TM, :] = rj

        def attn_group(base):
            q = [q_ref[j, base:base + RG, :] for j in range(NL)]
            ls = []
            for w in range(WIN):
                off = base + HALO - DIL * w
                t = q[0] * k_ref[0, off:off + RG, :]
                for j in range(1, NL):
                    t = t + q[j] * k_ref[j, off:off + RG, :]
                t = t + pltpu.roll(t, 64, 1)
                t = t + pltpu.roll(t, 32, 1)
                if base < DIL * w:
                    row = jax.lax.broadcasted_iota(jnp.int32, (RG, 128), 0) + base
                    t = jnp.where(row >= DIL * w, t, -1e9)
                ls.append(t)
            m = ls[0]
            for w in range(1, WIN):
                m = jnp.maximum(m, ls[w])
            ps = [jnp.exp2(l - m) for l in ls]
            s = ps[0]
            for w in range(1, WIN):
                s = s + ps[w]
            inv = 1.0 / s
            for j in range(NL):
                acc = ps[0] * v_ref[j, base + HALO:base + HALO + RG, :]
                for w in range(1, WIN):
                    off = base + HALO - DIL * w
                    acc = acc + ps[w] * v_ref[j, off:off + RG, :]
                o_ref[base:base + RG, j * 128:(j + 1) * 128] = (acc * inv).astype(bf16)

        def attn_block(i):
            for g in range(TM // RG):
                attn_group(i * TM + g * RG)

        gw = gw_ref[...].astype(f32).reshape(1, D)
        wr = wr_ref[...].astype(f32).reshape(1, D)

        def out_block(i):
            a = jnp.dot(o_ref[i * TM:(i + 1) * TM, :], wop_ref[...], preferred_element_type=f32)
            x = x_v[i * TM:(i + 1) * TM, :].astype(f32)
            g = jax.nn.sigmoid(jnp.sum(x * gw, axis=-1, keepdims=True))
            out_v[i * TM:(i + 1) * TM, :] = (x + g * (a - x)).astype(bf16)

        def route():
            x = x_v[...].astype(f32)
            r = jnp.sum(x * wr, axis=-1, keepdims=True)
            r = r.astype(bf16).astype(f32)
            m = jnp.max(r, axis=0, keepdims=True)
            row = jax.lax.broadcasted_iota(jnp.int32, (S, 1), 0)
            idx = jnp.min(jnp.where(r == m, row, S), axis=0, keepdims=True)
            idx_ref[0] = idx[0, 0]
            return m

        def ffn(rmax):
            idx = idx_ref[0]
            t16 = pl.multiple_of((idx // 16) * 16, 16)
            xt = x_v[pl.ds(t16, 16), :]
            hg = jax.lax.dot_general(xt, wg_v[...], NT, preferred_element_type=f32)
            hu = jax.lax.dot_general(xt, wu_v[...], NT, preferred_element_type=f32)
            hh = (hg * jax.nn.sigmoid(hg) * hu).astype(bf16)
            y = jnp.dot(hh, wd_v[...], preferred_element_type=f32)
            xf = xt.astype(f32)
            g = jax.nn.sigmoid(jnp.sum(xf * gw, axis=-1, keepdims=True))
            y = y * jax.nn.sigmoid(rmax) * (1.0 - g)
            row = jax.lax.broadcasted_iota(jnp.int32, (16, D), 0) + t16
            y_ref[...] = jnp.where(row == idx, y, 0.0)

        def patch(lo, hi):
            idx = idx_ref[0]
            @pl.when(jnp.logical_and(idx >= lo, idx < hi))
            def _():
                t16 = pl.multiple_of((idx // 16) * 16, 16)
                out_v[pl.ds(t16, 16), :] = (out_v[pl.ds(t16, 16), :].astype(f32) + y_ref[...]).astype(bf16)

        wcopy(0).wait()
        wcopy(2).start()
        prep_w(0)
        xcopy(0).wait()
        wcopy(1).wait()
        xcopy(1).start(); wocopy.start()
        qkv_part(0, 0); prep_w(1)
        wcopy(2).wait()
        for i in range(2, NB):
            xcopy(i).start()
        qkv_part(0, 1); prep_w(2)
        for c in fcopies:
            c.start()
        qkv_part(0, 2)
        rmax = None
        waited = {0}
        def xwait(i):
            if i not in waited:
                xcopy(i).wait(); waited.add(i)
        for i in range(NB + 1):
            if i + 1 < NB:
                xwait(i + 1)
            if i == 0:
                wocopy.wait(); prep_wo()
            if i == FFN_AT:
                for c in fcopies:
                    c.wait()
            if i + 1 < NB:
                for p in range(3):
                    qkv_part(i + 1, p)
            if i < NB:
                attn_block(i)
            if i >= 1:
                out_block(i - 1)
            if i == FFN_AT - 1:
                for ii in range(NB):
                    xwait(ii)
                rmax = route()
            if i == FFN_AT:
                ffn(rmax)
                patch(0, i * TM)
                for ii in range(i):
                    ocopy(ii).start()
            elif i > FFN_AT:
                patch((i - 1) * TM, i * TM)
                ocopy(i - 1).start()
        for i in range(NB):
            ocopy(i).wait()

    return kernel, NB


def build(TM=256, RG=64, FFN_AT=3):
    kernel, NB = make(TM, RG, FFN_AT)
    @jax.jit
    def fn(A_x, A_wqkv, A_wo, B_x, B_w_r, B_w_gate, B_w_up, B_w_down, gate_w):
        anyspec = pl.BlockSpec(memory_space=pltpu.HBM)
        vm = pl.BlockSpec(memory_space=pltpu.VMEM)
        return pl.pallas_call(
            kernel,
            in_specs=[anyspec, anyspec, anyspec, vm, anyspec, anyspec, anyspec, vm],
            out_specs=anyspec,
            out_shape=jax.ShapeDtypeStruct((1, S, D), bf16),
            scratch_shapes=[
                pltpu.VMEM((S, D), bf16), pltpu.VMEM((D, 3 * D), bf16), pltpu.VMEM((D, D), bf16),
                pltpu.VMEM((F, D), bf16), pltpu.VMEM((F, D), bf16), pltpu.VMEM((F, D), bf16),
                pltpu.VMEM((S, D), bf16),
                pltpu.VMEM((4 * NL, D, 128), f32), pltpu.VMEM((3 * D, D), bf16), pltpu.VMEM((D, D), bf16),
                pltpu.VMEM((NL, S, 128), f32), pltpu.VMEM((NL, S + HALO, 128), f32), pltpu.VMEM((NL, S + HALO, 128), f32),
                pltpu.VMEM((S, D), bf16), pltpu.VMEM((16, D), f32), pltpu.SMEM((1,), jnp.int32),
                pltpu.SemaphoreType.DMA((4,)), pltpu.SemaphoreType.DMA((NB,)),
                pltpu.SemaphoreType.DMA((3,)), pltpu.SemaphoreType.DMA((NB,)),
            ],
            compiler_params=pltpu.CompilerParams(vmem_limit_bytes=110 * 2**20),
        )(A_x, A_wqkv, A_wo, B_w_r, B_w_gate.T, B_w_up.T, B_w_down, gate_w)
    return fn


_impl = build()


@jax.jit
def pallas_gated_mix__sliding_local_dilated__moe_arch_mod__prompt_kernel(
    A_x: jax.Array,
    A_wqkv: jax.Array,
    A_wo: jax.Array,
    B_x: jax.Array,
    B_w_r: jax.Array,
    B_w_gate: jax.Array,
    B_w_up: jax.Array,
    B_w_down: jax.Array,
    gate_w: jax.Array,
):
    return _impl(A_x, A_wqkv, A_wo, B_x, B_w_r, B_w_gate, B_w_up, B_w_down, gate_w)
```

```python
import functools, math
import jax
import jax.numpy as jnp
import jax.experimental.pallas as pl
import jax.experimental.pallas.tpu as pltpu

S, D, H, DH, WIN, DIL, F = 2048, 640, 32, 20, 8, 2, 1728
NL = D // 128
HALO = 16
TM = 256
NB = S // TM
f32, bf16, u32, i32 = jnp.float32, jnp.bfloat16, jnp.uint32, jnp.int32
LOG2E = math.log2(math.e)
QSCALE = (DH ** -0.5) * LOG2E
NT = (((1,), (1,)), ((), ()))


def _recip(s):
    inv = pl.reciprocal(s, approx=True)
    return inv * (2.0 - s * inv)


def _sigmoid(x):
    return 0.5 * jnp.tanh(0.5 * x) + 0.5


def make(PROF=False, XG=32, FG=32, OUTTOK=2, RELD=4, TD=1, NH=2, UA=56, ORDER=(3, 2, 1), LAG=1, TKT=4, FINE=True, NC=32, ND=32, RESTOK=False, MID=0, CHAIN=0, NXB=3, NXC=4, NB1=5, NHALF=2, FR0=0.2, WTOK=1, TDO=2, CEND=3, EQ=0.89, WALL=False):
    RG = 8 * NH
    NU = S // RG

    def kernel(x_hbm, wqkv_hbm, wo_hbm, wr_hbm, wg_hbm, wu_hbm, wd_hbm, gw_hbm, out_hbm,
               x_v, wqkv_v, wo_v, wg_v, wu_v, wd_v, out_v, wr_ref, gw_ref,
               t_ref, wp_ref, wop_ref, xp_ref, q_ref, k_ref, v_ref, o_ref, g_ref, h_ref,
               sem):
        def wcopy(p, sm):
            return pltpu.make_async_copy(wqkv_hbm.at[:, p * D:(p + 1) * D], wqkv_v.at[:, p * D:(p + 1) * D], sem.at[sm])
        def xcopy(i, sm):
            return pltpu.make_async_copy(x_hbm.at[0, i * TM:(i + 1) * TM, :], x_v.at[i * TM:(i + 1) * TM, :], sem.at[sm])
        def ocopy(r0, n, c0, m):
            return pltpu.make_async_copy(out_v.at[r0:r0 + n, c0:c0 + m], out_hbm.at[0, r0:r0 + n, c0:c0 + m], sem.at[5])
        def w0piece(kt):
            return pltpu.make_async_copy(wqkv_hbm.at[kt * 128:(kt + 1) * 128, 0:D], wqkv_v.at[kt * 128:(kt + 1) * 128, 0:D],
                                         sem.at[6 if kt < 3 else 7])
        grpA = [xcopy(0, 0), pltpu.make_async_copy(wr_hbm, wr_ref, sem.at[0]),
                pltpu.make_async_copy(gw_hbm, gw_ref, sem.at[0])]
        w0p = [w0piece(kt) for kt in range(NL)]
        grpB = [xcopy(i, 1) for i in range(1, NXB + 1)]
        grpC = [wcopy(1, 2), wcopy(2, 2)] + [xcopy(i, 2) for i in range(NXB + 1, NXC + 1)]
        grpE = ([xcopy(i, 3) for i in range(NXC + 1, NB)] + [pltpu.make_async_copy(wo_hbm, wo_v, sem.at[3])]
                + [pltpu.make_async_copy(a, b, sem.at[3]) for (a, b) in ((wg_hbm, wg_v), (wu_hbm, wu_v), (wd_hbm, wd_v))])
        outs = []
        def start(g):
            for c in g: c.start()
        def wait(g):
            for c in g: c.wait()

        class _NS:
            def __init__(self, n): self.c = jax.named_scope(n) if PROF else None
            def __enter__(self):
                if self.c: self.c.__enter__()
            def __exit__(self, *a):
                if self.c: self.c.__exit__(*a)
        ns = _NS

        start(w0p); start(grpA); start(grpB)
        cst = {}
        def load_consts():
            cst["gw"] = jnp.broadcast_to(gw_ref[...].astype(f32).reshape(1, D), (8, D))
            cst["wr"] = jnp.broadcast_to(wr_ref[...].astype(f32).reshape(1, D), (8, D))
            cst["never"] = jnp.abs(cst["gw"][:, 0:128]) < 0.0

        for j in range(NL):
            k_ref[j, 0:HALO, :] = jnp.zeros((HALO, 128), f32)
            v_ref[j, 0:HALO, :] = jnp.zeros((HALO, 128), f32)

        delayq = []
        pending = []

        chainq = []
        taskno = [0]
        def tok(v, new=False, anchor=False):
            v = pltpu.bitcast(v, u32) if v.dtype != u32 else v
            if CHAIN and not anchor:
                if chainq and chainq[-1][0] == taskno[0]:
                    chainq[-1][1] = chainq[-1][1] | v
                else:
                    chainq.append([taskno[0], v])
                return
            if pending and not new:
                pending[-1] = pending[-1] | v
            else:
                pending.append(v)

        def with_tok(lhs_u32):
            delayq.append(list(pending)); pending.clear()
            toks = delayq.pop(0) if len(delayq) > TD else []
            if not toks:
                return lhs_u32
            ng = lhs_u32.shape[0] // 8
            slots = {}
            for n, t in enumerate(toks):
                r = (n * ng) // len(toks)
                slots[r] = t if r not in slots else slots[r] | t
            rows, prev = [], 0
            for r in sorted(slots):
                if r > prev:
                    rows.append(lhs_u32[prev * 8:r * 8, :])
                pieces = []
                if TKT > 0:
                    pieces.append(lhs_u32[r * 8:(r + 1) * 8, 0:TKT * 128])
                pieces.append(jnp.where(cst["never"], slots[r], lhs_u32[r * 8:(r + 1) * 8, TKT * 128:(TKT + 1) * 128]))
                if TKT < NL - 1:
                    pieces.append(lhs_u32[r * 8:(r + 1) * 8, (TKT + 1) * 128:])
                rows.append(jnp.concatenate(pieces, axis=1))
                prev = r + 1
            if prev < ng:
                rows.append(lhs_u32[prev * 8:, :])
            return jnp.concatenate(rows, axis=0)

        def res_tok(r):
            delayq.append(list(pending)); pending.clear()
            toks = delayq.pop(0) if len(delayq) > TD else []
            if not toks:
                return r
            ng = r.shape[0] // 8
            slots = {}
            for n, t in enumerate(toks):
                g = (n * ng) // len(toks)
                slots[g] = t if g not in slots else slots[g] | t
            rows, prev = [], 0
            for g in sorted(slots):
                if g > prev:
                    rows.append(r[prev * 8:g * 8, :])
                rows.append(jnp.where(cst["never"], pltpu.bitcast(slots[g], f32), r[g * 8:(g + 1) * 8, :]))
                prev = g + 1
            if prev < ng:
                rows.append(r[prev * 8:, :])
            return jnp.concatenate(rows, axis=0)

        ident = lambda v: v
        lhs_tok = with_tok if WTOK < 2 else ident
        lhs_tok_o = with_tok if WTOK < 1 else ident
        def w_tok(w, qkv):
            if WTOK < (2 if qkv else 1):
                return w
            if qkv:
                return with_tok(w)
            delayq.append(list(pending)); pending.clear()
            toks = delayq.pop(0) if len(delayq) > TDO else []
            if not toks:
                return w
            slots = {}
            for n, t in enumerate(toks):
                g = TKT * 8 + (n * 8) // len(toks) if not WALL else (n * 40) // len(toks)
                slots[g] = t if g not in slots else slots[g] | t
            rows, prev = [], 0
            for g in sorted(slots):
                if g > prev:
                    rows.append(w[prev * 8:g * 8, :])
                rows.append(jnp.where(cst["never"], slots[g], w[g * 8:(g + 1) * 8, :]))
                prev = g + 1
            if prev * 8 < w.shape[0]:
                rows.append(w[prev * 8:, :])
            return jnp.concatenate(rows, axis=0)
        if not RESTOK:
            res_tok = lambda v: v

        rel = []
        relcache = {}
        def released(v):
            if not (RELD and len(rel) >= RELD):
                return v
            r = rel[-RELD]
            if CHAIN:
                key = (taskno[0], len(rel))
                if relcache.get("key") != key:
                    ru = pltpu.bitcast(r, u32)
                    while chainq and chainq[0][0] <= taskno[0] - CHAIN:
                        ru = ru | chainq.pop(0)[1]
                    relcache["key"] = key; relcache["val"] = pltpu.bitcast(ru, f32)
                r = relcache["val"]
            r = r if v.dtype == f32 else pltpu.bitcast(r, v.dtype)
            rows = []
            for a in range(v.shape[0] // 8):
                rows.append(jnp.concatenate(
                    [jnp.where(cst["never"], r, v[a * 8:(a + 1) * 8, b * 128:(b + 1) * 128]) for b in range(v.shape[1] // 128)],
                    axis=1))
            return jnp.concatenate(rows, axis=0)

        def prep_w(p, kt):
            w = wqkv_v[kt * 128:(kt + 1) * 128, p * D:(p + 1) * D]
            t_ref[p * NL + kt] = w.T.astype(f32)
            for d in range(DH):
                r0 = (p * D + d * H) // 2
                wp_ref[r0:r0 + H // 2, kt * 128:(kt + 1) * 128] = pltpu.bitcast(
                    t_ref[p * NL + kt, pl.ds(d, H, stride=DH), :].astype(bf16), u32)

        def prep_wo(kt):
            w = pltpu.bitcast(released(pltpu.bitcast(wo_v[:, kt * 128:(kt + 1) * 128], u32)), bf16)
            t_ref[3 * NL + kt] = w.astype(f32)
            for d in range(DH):
                r0 = d * H // 2
                val = pltpu.bitcast(t_ref[3 * NL + kt, pl.ds(d, H, stride=DH), :].astype(bf16), u32)
                wop_ref[r0:r0 + H // 2, kt * 128:(kt + 1) * 128] = val

        def repack_x(r0, n):
            xp_ref[r0 // 2:(r0 + n) // 2, :] = released(pltpu.bitcast(x_v[r0:r0 + n, :], u32))

        def qkv_chunk(r0, n, p, j):
            xb = pltpu.bitcast(lhs_tok(xp_ref[r0 // 2:(r0 + n) // 2, :]), bf16)
            w0 = (p * D + j * 128) // 2
            w = pltpu.bitcast(w_tok(wp_ref[w0:w0 + 64, :], True), bf16)
            rj = jax.lax.dot_general(xb, w, NT, preferred_element_type=f32)
            rel.append(rj[n - 8:, :])
            rj = res_tok(rj)
            if p == 0:
                q_ref[j, r0:r0 + n, :] = rj * QSCALE
            else:
                ref = k_ref if p == 1 else v_ref
                ref[j, HALO + r0:HALO + r0 + n, :] = rj

        late = []
        def out_chunk(r0, n, j, dma):
            while len(late) >= OUTTOK:
                tok(late.pop(0), new=True, anchor=True)
            if NH == 2:
                ob = o_ref[r0 // 2:(r0 + n) // 2, :]
            else:
                ob = pltpu.bitcast(o_ref[r0:r0 + n, :], u32)
            ob = pltpu.bitcast(lhs_tok_o(ob), bf16)
            w = pltpu.bitcast(w_tok(wop_ref[:, j * 128:(j + 1) * 128], False), bf16)
            a = jnp.dot(ob, w, preferred_element_type=f32)
            rel.append(a[n - 8:, :])
            a = res_tok(a)
            x = x_v[r0:r0 + n, j * 128:(j + 1) * 128].astype(f32)
            g = g_ref[r0:r0 + n, :]
            res = x + g * (a - x)
            out_v[r0:r0 + n, j * 128:(j + 1) * 128] = res.astype(bf16)
            late.append(res[n - 8:, :])
            if dma is not None:
                c = ocopy(*dma)
                c.start(); outs.append(c)

        NE = WIN + 4 * (NH - 1)
        def uses(e):
            return [(a, e - 4 * (NH - 1 - a)) for a in range(NH) if 0 <= e - 4 * (NH - 1 - a) < WIN]

        def s1(base):
            q = [[released(q_ref[j, base + 8 * a:base + 8 * a + 8, :]) for j in range(NL)] for a in range(NH)]
            ts = {}
            for e in range(NE):
                off = base + HALO + 8 * (NH - 1) - DIL * e
                acc = {}
                for j in range(NL):
                    kk = k_ref[j, off:off + 8, :]
                    for (a, w) in uses(e):
                        pr = q[a][j] * kk
                        acc[a, w] = pr if j == 0 else acc[a, w] + pr
                for key, t in acc.items():
                    ts[key] = (t, pltpu.roll(t, 64, 1))
            return ts

        def s2(ts):
            us = {}
            for key, (t, r) in ts.items():
                u = t + r
                us[key] = (u, pltpu.roll(u, 32, 1))
            return us

        def s3(base, us):
            ps, inv = {}, {}
            for a in range(NH):
                ls = []
                for w in range(WIN):
                    u, rr = us[a, w]
                    t = u + rr
                    if base + 8 * a < DIL * w:
                        row = jax.lax.broadcasted_iota(i32, (8, 128), 0) + (base + 8 * a)
                        t = jnp.where(row >= DIL * w, t, -1e9)
                    ls.append(t)
                m = jnp.maximum(jnp.maximum(jnp.maximum(ls[0], ls[1]), jnp.maximum(ls[2], ls[3])),
                                jnp.maximum(jnp.maximum(ls[4], ls[5]), jnp.maximum(ls[6], ls[7])))
                p = [jnp.exp2(l - m) for l in ls]
                s = ((p[0] + p[1]) + (p[2] + p[3])) + ((p[4] + p[5]) + (p[6] + p[7]))
                inv[a] = _recip(s)
                if MID >= 2:
                    tok(m, new=True)
                if MID >= 1:
                    tok(inv[a], new=True)
                for w in range(WIN):
                    ps[a, w] = p[w]
            for j in range(NL):
                acc = {}
                for e in range(NE):
                    off = base + HALO + 8 * (NH - 1) - DIL * e
                    vv = v_ref[j, off:off + 8, :]
                    for (a, w) in uses(e):
                        pr = ps[a, w] * vv
                        acc[a] = pr if a not in acc else acc[a] + pr
                res = jnp.concatenate([acc[a] * inv[a] for a in range(NH)], axis=0).astype(bf16)
                if NH == 2:
                    res = pltpu.bitcast(res, u32)
                    o_ref[base // 2:base // 2 + 8, j * 128:(j + 1) * 128] = res
                    tok(res, new=(j == 0 or FINE))
                else:
                    o_ref[base:base + RG, j * 128:(j + 1) * 128] = res
                    tok(acc[0] * inv[0], new=(j == 0 or FINE))

        T, U = {}, {}
        def attn_step(g):
            for stage in ORDER:
                if stage == 1 and g < NU:
                    T[g] = s1(g * RG)
                if stage == 2 and 0 <= g - LAG < NU:
                    U[g - LAG] = s2(T.pop(g - LAG))
                if stage == 3 and 0 <= g - 2 * LAG < NU:
                    s3((g - 2 * LAG) * RG, U.pop(g - 2 * LAG))

        st = {}
        def gate_route(r0, n):
            gw_, wr_ = released(cst["gw"]), released(cst["wr"])
            for r in range(r0, r0 + n, 8):
                x = x_v[r:r + 8, :].astype(f32)
                gl = jnp.sum(x * gw_, axis=-1, keepdims=True)
                rl = jnp.sum(x * wr_, axis=-1, keepdims=True)
                g = _sigmoid(jnp.broadcast_to(gl, (8, 128)))
                g_ref[r:r + 8, :] = g
                tok(g, new=(r == r0))
                rl = jnp.broadcast_to(rl, (8, 128)).astype(bf16).astype(f32)
                if r == 0:
                    st["m"] = rl
                    st["i"] = jnp.zeros((8, 128), i32)
                else:
                    better = rl > st["m"]
                    st["m"] = jnp.where(better, rl, st["m"])
                    st["i"] = jnp.where(better, r, st["i"])
            tok(st["m"]); tok(st["i"])

        def finish_route():
            m8, i8 = st["m"], st["i"] + jax.lax.broadcasted_iota(i32, (8, 128), 0)
            m = jnp.max(m8, axis=0, keepdims=True)
            idxv = jnp.min(jnp.where(m8 == m, i8, S), axis=0, keepdims=True)
            idx = jnp.min(idxv)
            idx = jnp.clip(idx, 0, S - 1)
            t16 = pl.multiple_of((idx // 16) * 16, 16)
            xt = x_v[pl.ds(t16, 16), :].astype(f32)
            row = jax.lax.broadcasted_iota(i32, (16, D), 0) + t16
            sel = row == idx
            xs = jnp.sum(jnp.where(sel, xt, 0.0), axis=0, keepdims=True)
            st.update(rs=_sigmoid(m), t16=t16, idx=idx, xs=jnp.broadcast_to(xs, (8, D)))

        def ffn_gate(r0, n):
            xs = released(st["xs"])
            for r in range(r0, r0 + n, 8):
                hg = jnp.sum(wg_v[r:r + 8, :].astype(f32) * xs, axis=-1, keepdims=True)
                hg = jnp.broadcast_to(hg, (8, 128))
                sg = hg * _sigmoid(hg)
                h_ref[r:r + 8, :] = sg
                tok(sg, new=(r == r0))

        def ffn_up_down(r0, n):
            xs = released(st["xs"])
            for r in range(r0, r0 + n, 8):
                hu = jnp.sum(wu_v[r:r + 8, :].astype(f32) * xs, axis=-1, keepdims=True)
                h = h_ref[r:r + 8, :] * jnp.broadcast_to(hu, (8, 128))
                wd = wd_v[r:r + 8, :].astype(f32)
                contrib = [wd[:, j * 128:(j + 1) * 128] * h for j in range(NL)]
                if r == 0:
                    st["y"] = contrib
                else:
                    st["y"] = [a + b for a, b in zip(st["y"], contrib)]
            for n_, v in enumerate(st["y"]):
                tok(v, new=(n_ == 0))

        def ffn_finish():
            y = jnp.concatenate([jnp.sum(v, axis=0, keepdims=True) * st["rs"] for v in st["y"]], axis=1)
            t16 = st["t16"]
            xt = x_v[pl.ds(t16, 16), :].astype(f32)
            row = jax.lax.broadcasted_iota(i32, (16, D), 0) + t16
            x_v[pl.ds(t16, 16), :] = jnp.where(row == st["idx"], xt + y, xt).astype(bf16)

        def region(mx, vp):
            vp = sorted(vp, key=lambda t: t[0])
            n, k = len(mx), 0
            for c, chunk in enumerate(mx):
                lim = (c + 0.5) / n
                while k < len(vp) and vp[k][0] < lim:
                    taskno[0] += 1
                    vp[k][1](); k += 1
                chunk()
            while k < len(vp):
                vp[k][1](); k += 1
            pending.clear(); rel.clear(); delayq.clear(); chainq.clear()

        P = functools.partial
        def part(i, p):
            return [P(qkv_chunk, i * TM, TM, p, j) for j in range(NL)]
        def halves(i, p, j):
            return [P(qkv_chunk, i * TM, TM // 2, p, j), P(qkv_chunk, i * TM + TM // 2, TM // 2, p, j)]
        def spread(tasks, lo, hi):
            n = len(tasks)
            return [(lo + (hi - lo) * (t + 1) / n, task) for t, task in enumerate(tasks)]

        with ns("A"):
            wait(w0p[:3])
            start(grpC)
            for kt in range(3):
                prep_w(0, kt)
            wait(w0p[3:])
            for kt in range(3, NL):
                prep_w(0, kt)
            wait(grpA)
            load_consts()
            repack_x(0, TM)
            region(part(0, 0)[:NB1], spread([P(gate_route, r, XG) for r in range(0, TM, XG)], 0.0, 1.0))
        with ns("B"):
            wait(grpB)
            start(grpE)
            repack_x(TM, TM)
            mx = part(0, 0)[NB1:] + sum([part(i, 0) for i in range(1, NXB + 1)], [])
            vp = spread([P(gate_route, r, XG) for r in range(TM, (NXB + 1) * TM, XG)], 0.1, 1.0)
            vp += spread([P(repack_x, r, 64) for r in range(2 * TM, (NXB + 1) * TM, 64)], 0.0, 0.25)
            region(mx, vp)
        with ns("C"):
            wait(grpC)
            repack_x((NXB + 1) * TM, TM)
            for kt in range(NL):
                prep_w(1, kt)
            for kt in range(NL):
                prep_w(2, kt)
            allq = part(NXB + 1, 0) + part(0, 1) + part(0, 2)
            for i in range(NXB + 2, NXC + 1):
                allq += part(i, 0)
            navail = {0: 15}
            for i in range(1, NXC + 1):
                allq += part(i, 1) + part(i, 2)
                navail[i] = len(allq)
            nc = len(allq) // 4 * 4
            for i in range(NXC + 1, NB):
                allq += part(i, 0) + part(i, 1) + part(i, 2)
                navail[i] = len(allq)
            mx = allq[:nc]
            upb = TM // RG
            ua = UA * 2 // NH
            vp = []
            for g in range(ua):
                pos = (16 + (nc - CEND - 16) * (g + 1) / ua)
                pos = max(pos, navail[g // upb] + 1)
                vp.append((pos / nc, P(attn_step, g)))
            vp += spread([P(gate_route, r, XG) for r in range((NXB + 1) * TM, (NXC + 1) * TM, XG)], 0.05, 0.3)
            vp += spread([P(repack_x, r, 64) for r in range((NXB + 2) * TM, (NXC + 1) * TM, 64)], 0.05, 0.2)
            region(mx, vp)
        with ns("E"):
            wait(grpE)
            repack_x((NXC + 1) * TM, TM)
            mx = allq[nc:]
            nq = len(mx)
            for i in range(NB - 1):
                mx += [P(out_chunk, i * TM, TM, j, (i * TM, TM, 0, D) if j == NL - 1 else None) for j in range(NL)]
            n_before_last = len(mx)
            r7 = (NB - 1) * TM
            hm = TM // 2
            nfull = NL - NHALF
            mx += [P(out_chunk, r7, TM, j, (r7, TM, 0, nfull * 128) if j == nfull - 1 else None) for j in range(nfull)]
            for h in range(2):
                mx += [P(out_chunk, r7 + h * hm, hm, j, (r7 + h * hm, hm, nfull * 128, NHALF * 128) if j == NL - 1 else None)
                       for j in range(nfull, NL)]
            n = len(mx)
            vp = []
            rest = list(range(ua, NU + 2 * LAG))
            n1 = int(round(EQ * nq))
            for t, g in enumerate(rest):
                if t < n1:
                    pos = nq * (t + 1) / n1
                else:
                    pos = nq + (n_before_last - 0.6 - nq) * (t + 1 - n1) / (len(rest) - n1)
                pos = max(pos, navail[min(g, NU - 1) // upb] - nc + 1)
                vp.append((pos / n, P(attn_step, g)))
            f0 = FR0 * nq
            vp += spread([P(gate_route, r, XG) for r in range((NXC + 1) * TM, S, XG)], 0.0, (f0 - 1) / n)
            vp += spread([P(repack_x, r, 64) for r in range((NXC + 2) * TM, S, 64)], 0.0, 8 / n)
            vp += [(f0 / n, finish_route)]
            f1 = f0 + 0.4 * (nq - f0)
            vp += spread([P(ffn_gate, r, FG) for r in range(0, F, FG)], (f0 + 1) / n, f1 / n)
            vp += spread([P(ffn_up_down, r, FG) for r in range(0, F, FG)], f1 / n, (nq - 2) / n)
            vp += spread([P(prep_wo, kt) for kt in range(NL)], 0.1 * nq / n, 0.9 * nq / n)
            vp += [((nq - 1) / n, ffn_finish)]
            region(mx, vp)
        with ns("F"):
            wait(outs)

    return kernel, NH


def build(**kw):
    kernel, NH = make(**kw)
    @jax.jit
    def fn(A_x, A_wqkv, A_wo, B_x, B_w_r, B_w_gate, B_w_up, B_w_down, gate_w):
        anyspec = pl.BlockSpec(memory_space=pltpu.HBM)
        vm = pl.BlockSpec(memory_space=pltpu.VMEM)
        return pl.pallas_call(
            kernel,
            in_specs=[anyspec] * 8,
            out_specs=anyspec,
            out_shape=jax.ShapeDtypeStruct((1, S, D), bf16),
            scratch_shapes=[
                pltpu.VMEM((S, D), bf16), pltpu.VMEM((D, 3 * D), bf16), pltpu.VMEM((D, D), bf16),
                pltpu.VMEM((F, D), bf16), pltpu.VMEM((F, D), bf16), pltpu.VMEM((F, D), bf16),
                pltpu.VMEM((S, D), bf16), pltpu.VMEM((D,), bf16), pltpu.VMEM((D,), bf16),
                pltpu.VMEM((4 * NL, D, 128), f32), pltpu.VMEM((3 * D // 2, D), u32), pltpu.VMEM((D // 2, D), u32),
                pltpu.VMEM((S // 2, D), u32),
                pltpu.VMEM((NL, S, 128), f32), pltpu.VMEM((NL, S + HALO, 128), f32), pltpu.VMEM((NL, S + HALO, 128), f32),
                pltpu.VMEM((S // 2, D), u32) if NH == 2 else pltpu.VMEM((S, D), bf16),
                pltpu.VMEM((S, 128), f32), pltpu.VMEM((F, 128), f32),
                pltpu.SemaphoreType.DMA((8,)),
            ],
            compiler_params=pltpu.CompilerParams(vmem_limit_bytes=110 * 2**20),
        )(A_x, A_wqkv, A_wo, B_w_r, B_w_gate.T, B_w_up.T, B_w_down, gate_w)
    return fn


_impl = build()


@jax.jit
def pallas_gated_mix__sliding_local_dilated__moe_arch_mod__prompt_kernel(
    A_x: jax.Array,
    A_wqkv: jax.Array,
    A_wo: jax.Array,
    B_x: jax.Array,
    B_w_r: jax.Array,
    B_w_gate: jax.Array,
    B_w_up: jax.Array,
    B_w_down: jax.Array,
    gate_w: jax.Array,
):
    return _impl(A_x, A_wqkv, A_wo, B_x, B_w_r, B_w_gate, B_w_up, B_w_down, gate_w)
```

```python
import functools
import math

import jax
import jax.numpy as jnp
import jax.experimental.pallas as pl
import jax.experimental.pallas.tpu as pltpu

S, D, H, DH, WIN, DIL, F = 2048, 640, 32, 20, 8, 2, 1728
NL = D // 128
HALO = 16
TM = 256
NB = S // TM
RG = 16
NU = S // RG
NE = WIN + 4
f32, bf16, u32, i32 = jnp.float32, jnp.bfloat16, jnp.uint32, jnp.int32
LOG2E = math.log2(math.e)
QSCALE = (DH ** -0.5) * LOG2E
NEG = -1e9 * LOG2E
NT = (((1,), (1,)), ((), ()))


def _recip(s):
    inv = pl.reciprocal(s, approx=True)
    return inv * (2.0 - s * inv)


def _sigmoid(x):
    return 0.5 * jnp.tanh(0.5 * x) + 0.5


def make(XG=16, FG=16, OUTTOK=2, RELD=6, TD=2, TDO=2, UA=56, CEND=3, EQ=0.89, FR0=0.2, GAP=2, FE=2,
         QH=5, A0=1, KS=3, G0=2.0, G1=12.0, GBE=4):

    def kernel(x_hbm, wqkv_hbm, wo_hbm, wr_hbm, wg_hbm, wu_hbm, wd_hbm, gw_hbm, out_hbm,
               x_v, wqkv_v, wo_v, wg_v, wu_v, wd_v, out_v, wr_ref, gw_ref,
               t_ref, wp_ref, wop_ref, xp_ref, q_ref, k_ref, v_ref, o_ref, g_ref, g1_ref, h_ref,
               sem):
        P = functools.partial
        cp = pltpu.make_async_copy

        def wcopy(r0, r1, p, sm):
            return cp(wqkv_hbm.at[r0:r1, p * D:(p + 1) * D], wqkv_v.at[r0:r1, p * D:(p + 1) * D], sem.at[sm])

        def xcopy(i, sm):
            return cp(x_hbm.at[0, i * TM:(i + 1) * TM, :], x_v.at[i * TM:(i + 1) * TM, :], sem.at[sm])

        w0a = [wcopy(kt * 128, (kt + 1) * 128, 0, 0) for kt in range(KS)]
        grp_a = [xcopy(0, 2), cp(wr_hbm, wr_ref, sem.at[2]), cp(gw_hbm, gw_ref, sem.at[2])]
        grp_a2 = [wcopy(KS * 128, D, 0, 1), xcopy(1, 1)]
        grp_b = [xcopy(i, 3) for i in (2, 3)]
        grp_c = [wcopy(0, D, 1, 4), wcopy(0, D, 2, 4), xcopy(4, 4)]
        grp_e = [xcopy(i, 5) for i in (5, 6, 7)] + [
            cp(a, b, sem.at[5]) for a, b in ((wo_hbm, wo_v), (wg_hbm, wg_v), (wu_hbm, wu_v), (wd_hbm, wd_v))]
        outs = []

        def start(g):
            for c in g:
                c.start()

        def wait(g):
            for c in g:
                c.wait()

        done = set()

        def need(*keys):
            for k_ in keys:
                assert k_ in done, k_

        start(w0a); start(grp_a); start(grp_a2); start(grp_b)
        for j in range(NL):
            k_ref[j, 0:HALO, :] = jnp.zeros((HALO, 128), f32)
            v_ref[j, 0:HALO, :] = jnp.zeros((HALO, 128), f32)

        cst, pending, delayq, rel = {}, [], [], []

        def tok(v, new=False):
            v = v if v.dtype == u32 else pltpu.bitcast(v, u32)
            if pending and not new:
                pending[-1] = pending[-1] | v
            else:
                pending.append(v)

        def attach(a, delay, g0, ng, c0):
            delayq.append(list(pending)); pending.clear()
            toks = delayq.pop(0) if len(delayq) > delay else []
            if not toks:
                return a
            slots = {}
            for n, t in enumerate(toks):
                g = g0 + (n * ng) // len(toks)
                slots[g] = t if g not in slots else slots[g] | t
            rows, prev = [], 0
            for g in sorted(slots):
                if g > prev:
                    rows.append(a[prev * 8:g * 8, :])
                last = jnp.where(cst["never"], slots[g], a[g * 8:(g + 1) * 8, c0 * 128:(c0 + 1) * 128])
                rows.append(jnp.concatenate([a[g * 8:(g + 1) * 8, 0:c0 * 128], last], axis=1) if c0 else last)
                prev = g + 1
            if prev * 8 < a.shape[0]:
                rows.append(a[prev * 8:, :])
            return jnp.concatenate(rows, axis=0)

        def released(v):
            if len(rel) < RELD:
                return v
            r = rel[-RELD] if v.dtype == f32 else pltpu.bitcast(rel[-RELD], v.dtype)
            return jnp.concatenate([
                jnp.concatenate([jnp.where(cst["never"], r, v[a * 8:(a + 1) * 8, b * 128:(b + 1) * 128])
                                 for b in range(v.shape[1] // 128)], axis=1)
                for a in range(v.shape[0] // 8)], axis=0)

        def prep_w(p, kt):
            wt = wqkv_v[kt * 128:(kt + 1) * 128, p * D:(p + 1) * D].T.astype(f32)
            t_ref[p * NL + kt] = wt * QSCALE if p == 0 else wt
            for d in range(DH):
                r0 = (p * D + d * H) // 2
                wp_ref[r0:r0 + H // 2, kt * 128:(kt + 1) * 128] = pltpu.bitcast(
                    t_ref[p * NL + kt, pl.ds(d, H, stride=DH), :].astype(bf16), u32)
            done.add(("wp", p, kt))

        def prep_wo(j):
            w = pltpu.bitcast(released(pltpu.bitcast(wo_v[:, j * 128:(j + 1) * 128], u32)), bf16)
            t_ref[3 * NL + j] = w.astype(f32)
            for d in range(DH):
                wop_ref[d * H // 2:(d + 1) * H // 2, j * 128:(j + 1) * 128] = pltpu.bitcast(
                    t_ref[3 * NL + j, pl.ds(d, H, stride=DH), :].astype(bf16), u32)
            done.add(("wop", j))

        def repack_x(r0, n):
            assert "patched" not in done
            xp_ref[r0 // 2:(r0 + n) // 2, :] = released(pltpu.bitcast(x_v[r0:r0 + n, :], u32))
            done.update(("xp", r) for r in range(r0, r0 + n, 8))

        def qkv_chunk(r0, n, p, j, k0=0, k1=NL):
            need(*[("xp", r) for r in range(r0, r0 + n, 8)], *[("wp", p, kt) for kt in range(k0, k1)])
            xb = pltpu.bitcast(attach(xp_ref[r0 // 2:(r0 + n) // 2, k0 * 128:k1 * 128], TD, 0, n // 16, k1 - k0 - 1), bf16)
            w0 = (p * D + j * 128) // 2
            r = jax.lax.dot_general(xb, pltpu.bitcast(wp_ref[w0:w0 + 64, k0 * 128:k1 * 128], bf16), NT,
                                    preferred_element_type=f32)
            rel.append(r[n - 8:, :])
            if p == 0:
                first = k1 - k0 < NL and ("qa", j, r0) not in done
                if k1 - k0 < NL and not first:
                    need(*[("qa", j, r_) for r_ in range(r0, r0 + n, 8)])
                    r = r + q_ref[j, r0:r0 + n, :]
                q_ref[j, r0:r0 + n, :] = r
            else:
                first = False
                (k_ref if p == 1 else v_ref)[j, HALO + r0:HALO + r0 + n, :] = r
            done.update(("qa" if first else "qkv"[p], j, r_) for r_ in range(r0, r0 + n, 8))

        late = []

        def out_chunk(r0, n, j, dma):
            need("patched", ("wop", j), *[("o", r) for r in range(r0, r0 + n, RG)])
            while len(late) >= OUTTOK:
                tok(late.pop(0), new=True)
            ob = pltpu.bitcast(o_ref[r0 // 2:(r0 + n) // 2, :], bf16)
            w = pltpu.bitcast(attach(wop_ref[:, j * 128:(j + 1) * 128], TDO, (NL - 1) * 8, 8, 0), bf16)
            a = jnp.dot(ob, w, preferred_element_type=f32)
            rel.append(a[n - 8:, :])
            res = x_v[r0:r0 + n, j * 128:(j + 1) * 128].astype(f32) * g1_ref[r0:r0 + n, :] + a
            out_v[r0:r0 + n, j * 128:(j + 1) * 128] = res.astype(bf16)
            late.append(res[n - 8:, :])
            done.update(("out", j, r) for r in range(r0, r0 + n, 8))
            if dma is not None:
                c0, m = dma
                need(*[("out", j_, r) for j_ in range(c0, c0 + m) for r in range(r0, r0 + n, 8)])
                c = cp(out_v.at[r0:r0 + n, c0 * 128:(c0 + m) * 128],
                       out_hbm.at[0, r0:r0 + n, c0 * 128:(c0 + m) * 128], sem.at[6])
                c.start(); outs.append(c)

        def uses(e):
            return [(a, e - 4 * (1 - a)) for a in range(2) if 0 <= e - 4 * (1 - a) < WIN]

        def window(name, base):
            need(*[(name, j, r) for j in range(NL) for r in range(max(base - HALO, 0), base + RG, 8)])

        def s1(base):
            window("k", base); need(*[("q", j, base + 8 * a) for j in range(NL) for a in range(2)])
            q = [[released(q_ref[j, base + 8 * a:base + 8 * a + 8, :]) for j in range(NL)] for a in range(2)]
            ts = {}
            for e in range(NE):
                off = base + HALO + 8 - DIL * e
                acc = {}
                for j in range(NL):
                    kk = k_ref[j, off:off + 8, :]
                    for (a, w) in uses(e):
                        pr = q[a][j] * kk
                        acc[a, w] = pr if j == 0 else acc[a, w] + pr
                for key, t in acc.items():
                    ts[key] = (t, pltpu.roll(t, 64, 1))
            return ts

        def s2(ts):
            us = {}
            for key, (t, r) in ts.items():
                u = t + r
                us[key] = (u, pltpu.roll(u, 32, 1))
            return us

        def s3(base, us):
            window("v", base); need(("g", base), ("g", base + 8))
            ps, inv = {}, []
            for a in range(2):
                ls = []
                for w in range(WIN):
                    u, r = us[a, w]
                    t = u + r
                    if base + 8 * a < DIL * w:
                        row = jax.lax.broadcasted_iota(i32, (8, 128), 0) + (base + 8 * a)
                        t = jnp.where(row >= DIL * w, t, NEG)
                    ls.append(t)
                m = jnp.maximum(jnp.maximum(jnp.maximum(ls[0], ls[1]), jnp.maximum(ls[2], ls[3])),
                                jnp.maximum(jnp.maximum(ls[4], ls[5]), jnp.maximum(ls[6], ls[7])))
                p = [jnp.exp2(l - m) for l in ls]
                inv.append(_recip(((p[0] + p[1]) + (p[2] + p[3])) + ((p[4] + p[5]) + (p[6] + p[7]))))
                for w in range(WIN):
                    ps[a, w] = p[w]
            scl = jnp.concatenate(inv, axis=0) * g_ref[base:base + RG, :]
            for j in range(NL):
                acc = {}
                for e in range(NE):
                    off = base + HALO + 8 - DIL * e
                    vv = v_ref[j, off:off + 8, :]
                    for (a, w) in uses(e):
                        pr = ps[a, w] * vv
                        acc[a] = pr if a not in acc else acc[a] + pr
                res = jnp.concatenate([acc[0], acc[1]], axis=0) * scl
                o_ref[base // 2:base // 2 + 8, j * 128:(j + 1) * 128] = pltpu.bitcast(res.astype(bf16), u32)
                tok(res[0:8, :], new=True); tok(res[8:16, :])
            done.add(("o", base))

        T, U = {}, {}

        def attn_step(g):
            if 0 <= g - 2 < NU:
                s3((g - 2) * RG, U.pop(g - 2))
            if 0 <= g - 1 < NU:
                U[g - 1] = s2(T.pop(g - 1))
            if g < NU:
                T[g] = s1(g * RG)

        st = {}

        def gate_route(r0, n):
            assert "patched" not in done and (r0 == 0 or ("g", r0 - 8) in done)
            gw, wr = released(cst["gw"]), released(cst["wr"])
            for r in range(r0, r0 + n, 8):
                x = x_v[r:r + 8, :].astype(f32)
                gl = jnp.sum(x * gw, axis=-1, keepdims=True)
                rl = jnp.sum(x * wr, axis=-1, keepdims=True)
                hh = 0.5 * jnp.tanh(0.5 * jnp.broadcast_to(gl, (8, 128)))
                g_ref[r:r + 8, :] = 0.5 + hh
                g1_ref[r:r + 8, :] = 0.5 - hh
                tok(hh, new=(r == r0))
                rl = jnp.broadcast_to(rl, (8, 128)).astype(bf16).astype(f32)
                if r == 0:
                    st["m"], st["i"] = rl, jnp.zeros((8, 128), i32)
                else:
                    better = rl > st["m"]
                    st["m"] = jnp.where(better, rl, st["m"])
                    st["i"] = jnp.where(better, r, st["i"])
                done.add(("g", r))
            tok(st["m"]); tok(st["i"])

        def finish_route():
            need(("g", S - 8))
            m8, i8 = st["m"], st["i"] + jax.lax.broadcasted_iota(i32, (8, 128), 0)
            m = jnp.max(m8, axis=0, keepdims=True)
            idx = jnp.clip(jnp.min(jnp.min(jnp.where(m8 == m, i8, S), axis=0, keepdims=True)), 0, S - 1)
            t16 = pl.multiple_of((idx // 16) * 16, 16)
            xt = x_v[pl.ds(t16, 16), :].astype(f32)
            row = jax.lax.broadcasted_iota(i32, (16, D), 0) + t16
            xs = jnp.sum(jnp.where(row == idx, xt, 0.0), axis=0, keepdims=True)
            st.update(rs=_sigmoid(m), t16=t16, idx=idx, xs=jnp.broadcast_to(xs, (8, D)))

        def ffn_gate(r0, n):
            xs = released(st["xs"])
            for r in range(r0, r0 + n, 8):
                hg = jnp.sum(wg_v[r:r + 8, :].astype(f32) * xs, axis=-1, keepdims=True)
                hg = jnp.broadcast_to(hg, (8, 128))
                sg = hg * _sigmoid(hg)
                h_ref[r:r + 8, :] = sg
                tok(sg, new=(r == r0))
                done.add(("h", r))

        def ffn_up_down(r0, n):
            xs = released(st["xs"])
            for r in range(r0, r0 + n, 8):
                need(("h", r))
                hu = jnp.sum(wu_v[r:r + 8, :].astype(f32) * xs, axis=-1, keepdims=True)
                h = h_ref[r:r + 8, :] * jnp.broadcast_to(hu, (8, 128))
                wd = wd_v[r:r + 8, :].astype(f32)
                c = [wd[:, j * 128:(j + 1) * 128] * h for j in range(NL)]
                st["y"] = c if r == 0 else [a + b for a, b in zip(st["y"], c)]
                done.add(("y", r))
            for n_, v in enumerate(st["y"]):
                tok(v, new=(n_ == 0))

        def ffn_finish():
            need(*[("y", r) for r in range(0, F, 8)], *[("xp", r) for r in range(0, S, 8)])
            y = jnp.concatenate([jnp.sum(v, axis=0, keepdims=True) * st["rs"] for v in st["y"]], axis=1)
            t16 = st["t16"]
            xt = x_v[pl.ds(t16, 16), :].astype(f32)
            row = jax.lax.broadcasted_iota(i32, (16, D), 0) + t16
            x_v[pl.ds(t16, 16), :] = jnp.where(row == st["idx"], xt + y, xt).astype(bf16)
            done.add("patched")

        def region(mx, vp):
            vp = sorted(vp, key=lambda t: t[0])
            k = 0
            for c, chunk in enumerate(mx):
                while k < len(vp) and vp[k][0] < c + 0.5:
                    vp[k][1](); k += 1
                chunk()
            for _, task in vp[k:]:
                task()
            pending.clear(); rel.clear(); delayq.clear()

        def part(i, p, js=range(NL), rows=TM, k0=0, k1=NL):
            return [P(qkv_chunk, i * TM + r, rows, p, j, k0, k1) for j in js for r in range(0, TM, rows)]

        def spread(fn, r0, r1, step, lo, hi):
            rs = list(range(r0, r1, step))
            return [(lo + (hi - lo) * (t + 1) / len(rs), P(fn, r, step)) for t, r in enumerate(rs)]

        wait(w0a)
        start(grp_c)
        cst["never"] = jnp.abs(wqkv_v[0:8, 0:128].astype(f32)) < 0.0
        for kt in range(KS):
            prep_w(0, kt)
        wait(grp_a)
        cst["gw"] = jnp.broadcast_to(gw_ref[...].astype(f32).reshape(1, D), (8, D))
        cst["wr"] = jnp.broadcast_to(wr_ref[...].astype(f32).reshape(1, D), (8, D))
        repack_x(0, TM)
        region(part(0, 0, range(4), TM, 0, KS) + part(0, 0, (4,), TM // 4, 0, KS), [])
        wait(grp_a2)
        start(grp_e)
        repack_x(TM, TM)
        for kt in range(KS, NL):
            prep_w(0, kt)
        mx = (part(1, 0, range(4), TM, 0, KS) + part(0, 0, range(NL), TM, KS, NL)
              + part(1, 0, range(NL), TM, KS, NL) + part(1, 0, (4,), TM // 4, 0, KS))
        region(mx, spread(gate_route, 0, TM, XG, G0, G1))
        wait(grp_b)
        repack_x(2 * TM, TM)
        mx = part(2, 0) + part(3, 0, (0, 1, 2)) + part(3, 0, (3, 4), TM // 2)
        n = len(mx)
        region(mx, spread(gate_route, TM, GBE * TM, XG, 1.0, n - 3) + spread(repack_x, 3 * TM, 4 * TM, 64, 0.0, 3.0))
        wait(grp_c)
        repack_x(4 * TM, TM)
        for p in (1, 2):
            for kt in range(NL):
                prep_w(p, kt)
        allq = part(4, 0)[:QH] + part(0, 1) + part(0, 2)
        avail = {0: len(allq)}
        allq += part(4, 0)[QH:]
        for i in range(1, 5):
            allq += part(i, 1) + part(i, 2)
            avail[i] = len(allq)
        nc = len(allq) // 4 * 4
        for i in range(5, NB):
            allq += part(i, 0) + part(i, 1) + part(i, 2)
            avail[i] = len(allq)
        upb = TM // RG
        a0 = avail[0] + A0
        vp = [(max(a0 + (nc - CEND - a0) * (g + 1) / UA, avail[g // upb] + 1), P(attn_step, g)) for g in range(UA)]
        vp += spread(gate_route, GBE * TM, 5 * TM, XG, 0.05 * nc, 0.3 * nc)
        region(allq[:nc], vp)
        wait(grp_e)
        repack_x(5 * TM, TM)
        mx = allq[nc:]
        nq = len(mx)
        for i in range(NB - 1):
            mx += [P(out_chunk, i * TM, TM, j, (0, NL) if j == NL - 1 else None) for j in range(NL)]
        nbl = len(mx)
        r7, hm = (NB - 1) * TM, TM // 2
        mx += [P(out_chunk, r7, TM, j, (0, 3) if j == 2 else None) for j in range(3)]
        mx += [P(out_chunk, r7 + h * hm, hm, j, (3, 2) if j == 4 else None) for h in range(2) for j in (3, 4)]
        rest = list(range(UA, NU + 2))
        n1 = int(round(EQ * nq))
        vp = []
        for t, g in enumerate(rest):
            pos = (nq - GAP) * (t + 1) / n1 if t < n1 else nq + (nbl - 0.6 - nq) * (t + 1 - n1) / (len(rest) - n1)
            vp.append((max(pos, avail[min(g, NU - 1) // upb] - nc + 1), P(attn_step, g)))
        f0 = FR0 * nq
        f1 = f0 + 0.4 * (nq - f0)
        vp += spread(gate_route, 5 * TM, S, XG, 0.0, f0 - 1)
        vp += spread(repack_x, 6 * TM, S, 64, 0.0, 8)
        vp += [(f0, finish_route)]
        vp += spread(ffn_gate, 0, F, FG, f0 + 1, f1)
        vp += spread(ffn_up_down, 0, F, FG, f1, nq - FE)
        vp += [(0.1 * nq + 0.8 * nq * (j + 1) / NL, P(prep_wo, j)) for j in range(NL)]
        vp += [(nq - FE + 1, ffn_finish)]
        region(mx, vp)
        wait(outs)

    return kernel


def build(**kw):
    kernel = make(**kw)

    @jax.jit
    def fn(A_x, A_wqkv, A_wo, B_x, B_w_r, B_w_gate, B_w_up, B_w_down, gate_w):
        hbm = pl.BlockSpec(memory_space=pltpu.MemorySpace.HBM)
        vm = pltpu.VMEM
        return pl.pallas_call(
            kernel,
            in_specs=[hbm] * 8,
            out_specs=hbm,
            out_shape=jax.ShapeDtypeStruct((1, S, D), bf16),
            scratch_shapes=[
                vm((S, D), bf16), vm((D, 3 * D), bf16), vm((D, D), bf16),
                vm((F, D), bf16), vm((F, D), bf16), vm((F, D), bf16),
                vm((S, D), bf16), vm((D,), bf16), vm((D,), bf16),
                vm((4 * NL, D, 128), f32), vm((3 * D // 2, D), u32), vm((D // 2, D), u32),
                vm((S // 2, D), u32),
                vm((NL, S, 128), f32), vm((NL, S + HALO, 128), f32), vm((NL, S + HALO, 128), f32),
                vm((S // 2, D), u32),
                vm((S, 128), f32), vm((S, 128), f32), vm((F, 128), f32),
                pltpu.SemaphoreType.DMA((7,)),
            ],
            compiler_params=pltpu.CompilerParams(vmem_limit_bytes=110 * 2**20),
        )(A_x, A_wqkv, A_wo, B_w_r, B_w_gate.T, B_w_up.T, B_w_down, gate_w)
    return fn


_impl = build()


@jax.jit
def pallas_gated_mix__sliding_local_dilated__moe_arch_mod__prompt_kernel(
    A_x: jax.Array,
    A_wqkv: jax.Array,
    A_wo: jax.Array,
    B_x: jax.Array,
    B_w_r: jax.Array,
    B_w_gate: jax.Array,
    B_w_up: jax.Array,
    B_w_down: jax.Array,
    gate_w: jax.Array,
):
    return _impl(A_x, A_wqkv, A_wo, B_x, B_w_r, B_w_gate, B_w_up, B_w_down, gate_w)
```

```python
import functools
import math

import jax
import jax.numpy as jnp
import jax.experimental.pallas as pl
import jax.experimental.pallas.tpu as pltpu

S, D, H, DH, WIN, DIL, F = 2048, 640, 32, 20, 8, 2, 1728
NL = D // 128
HALO = 16
TM = 256
NB = S // TM
RG = 16
NU = S // RG
NE = WIN + 4
f32, bf16, u32, i32 = jnp.float32, jnp.bfloat16, jnp.uint32, jnp.int32
LOG2E = math.log2(math.e)
QSCALE = (DH ** -0.5) * LOG2E
NEG = -1e9 * LOG2E
NT = (((1,), (1,)), ((), ()))


def _recip(s):
    inv = pl.reciprocal(s, approx=True)
    return inv * (2.0 - s * inv)


def _sigmoid(x):
    return 0.5 * jnp.tanh(0.5 * x) + 0.5


def make(XG=16, FG=16, OUTTOK=2, RELD=6, TD=2, TDO=2, UA=56, CEND=3, EQ=0.87, FR0=0.2, GAP=2, FE=2,
         QH=5, A0=1, KS=3, G0=2.0, G1=12.0, GBE=4):

    def kernel(x_hbm, wqkv_hbm, wo_hbm, wr_hbm, wg_hbm, wu_hbm, wd_hbm, gw_hbm, out_hbm,
               x_v, wqkv_v, wo_v, wg_v, wu_v, wd_v, out_v, wr_ref, gw_ref,
               t_ref, wp_ref, wop_ref, xp_ref, q_ref, k_ref, v_ref, o_ref, g_ref, g1_ref, h_ref,
               sem):
        P = functools.partial
        cp = pltpu.make_async_copy

        def wcopy(r0, r1, p, sm):
            return cp(wqkv_hbm.at[r0:r1, p * D:(p + 1) * D], wqkv_v.at[r0:r1, p * D:(p + 1) * D], sem.at[sm])

        def xcopy(i, sm):
            return cp(x_hbm.at[0, i * TM:(i + 1) * TM, :], x_v.at[i * TM:(i + 1) * TM, :], sem.at[sm])

        w0a = [wcopy(kt * 128, (kt + 1) * 128, 0, 0) for kt in range(KS)]
        grp_a = [xcopy(0, 2), cp(wr_hbm, wr_ref, sem.at[2]), cp(gw_hbm, gw_ref, sem.at[2])]
        grp_a2 = [wcopy(KS * 128, D, 0, 1), xcopy(1, 1)]
        grp_b = [xcopy(i, 3) for i in (2, 3)]
        grp_c = [wcopy(0, D, 1, 4), wcopy(0, D, 2, 4), xcopy(4, 4)]
        grp_e = [xcopy(i, 5) for i in (5, 6, 7)] + [
            cp(a, b, sem.at[5]) for a, b in ((wo_hbm, wo_v), (wg_hbm, wg_v), (wu_hbm, wu_v), (wd_hbm, wd_v))]
        outs = []

        def start(g):
            for c in g:
                c.start()

        def wait(g):
            for c in g:
                c.wait()

        done = set()

        def need(*keys):
            for k_ in keys:
                assert k_ in done, k_

        start(w0a); start(grp_a); start(grp_a2); start(grp_b)
        for j in range(NL):
            k_ref[j, 0:HALO, :] = jnp.zeros((HALO, 128), f32)
            v_ref[j, 0:HALO, :] = jnp.zeros((HALO, 128), f32)

        cst, pending, delayq, rel = {}, [], [], []

        def tok(v, new=False):
            v = v if v.dtype == u32 else pltpu.bitcast(v, u32)
            if pending and not new:
                pending[-1] = pending[-1] | v
            else:
                pending.append(v)

        def attach(a, delay, g0, ng, c0):
            delayq.append(list(pending)); pending.clear()
            toks = delayq.pop(0) if len(delayq) > delay else []
            if not toks:
                return a
            slots = {}
            for n, t in enumerate(toks):
                g = g0 + (n * ng) // len(toks)
                slots[g] = t if g not in slots else slots[g] | t
            rows, prev = [], 0
            for g in sorted(slots):
                if g > prev:
                    rows.append(a[prev * 8:g * 8, :])
                last = jnp.where(cst["never"], slots[g], a[g * 8:(g + 1) * 8, c0 * 128:(c0 + 1) * 128])
                rows.append(jnp.concatenate([a[g * 8:(g + 1) * 8, 0:c0 * 128], last], axis=1) if c0 else last)
                prev = g + 1
            if prev * 8 < a.shape[0]:
                rows.append(a[prev * 8:, :])
            return jnp.concatenate(rows, axis=0)

        def released(v):
            if len(rel) < RELD:
                return v
            r = rel[-RELD] if v.dtype == f32 else pltpu.bitcast(rel[-RELD], v.dtype)
            return jnp.where(cst["never"], r, v)

        def released2(v):
            if len(rel) < RELD:
                return v
            r = rel[-RELD] if v.dtype == f32 else pltpu.bitcast(rel[-RELD], v.dtype)
            reps = (v.shape[0] // 8, v.shape[1] // 128)
            return jnp.where(jnp.tile(cst["never"], reps), jnp.tile(r, reps), v)

        def prep_w(p, kt):
            t_ref[p * NL + kt] = wqkv_v[kt * 128:(kt + 1) * 128, p * D:(p + 1) * D].T.astype(f32)
            for d in range(DH):
                r0 = (p * D + d * H) // 2
                wp_ref[r0:r0 + H // 2, kt * 128:(kt + 1) * 128] = pltpu.bitcast(
                    t_ref[p * NL + kt, pl.ds(d, H, stride=DH), :].astype(bf16), u32)
            done.add(("wp", p, kt))

        def prep_wo(j):
            w = pltpu.bitcast(released2(pltpu.bitcast(wo_v[:, j * 128:(j + 1) * 128], u32)), bf16)
            t_ref[3 * NL + j] = w.astype(f32)
            for d in range(DH):
                wop_ref[d * H // 2:(d + 1) * H // 2, j * 128:(j + 1) * 128] = pltpu.bitcast(
                    t_ref[3 * NL + j, pl.ds(d, H, stride=DH), :].astype(bf16), u32)
            done.add(("wop", j))

        def repack_x(r0, n):
            assert "patched" not in done
            need(*[("x", r // TM) for r in range(r0, r0 + n, 8)])
            xp_ref[r0 // 2:(r0 + n) // 2, :] = released2(pltpu.bitcast(x_v[r0:r0 + n, :], u32))
            done.update(("xp", r) for r in range(r0, r0 + n, 8))

        def qkv_chunk(r0, n, p, j, k0=0, k1=NL):
            need(*[("xp", r) for r in range(r0, r0 + n, 8)], *[("wp", p, kt) for kt in range(k0, k1)])
            xb = pltpu.bitcast(attach(xp_ref[r0 // 2:(r0 + n) // 2, k0 * 128:k1 * 128], TD, 0, n // 16, k1 - k0 - 1), bf16)
            w0 = (p * D + j * 128) // 2
            r = jax.lax.dot_general(xb, pltpu.bitcast(wp_ref[w0:w0 + 64, k0 * 128:k1 * 128], bf16), NT,
                                    preferred_element_type=f32)
            rel.append(r[n - 8:, :])
            if p == 0:
                first = k1 - k0 < NL and ("qa", j, r0) not in done
                if k1 - k0 < NL and not first:
                    need(*[("qa", j, r_) for r_ in range(r0, r0 + n, 8)])
                    r = r + q_ref[j, r0:r0 + n, :]
                q_ref[j, r0:r0 + n, :] = r if first else r * QSCALE
            else:
                first = False
                (k_ref if p == 1 else v_ref)[j, HALO + r0:HALO + r0 + n, :] = r
            done.update(("qa" if first else "qkv"[p], j, r_) for r_ in range(r0, r0 + n, 8))

        late = []

        def out_chunk(r0, n, j, dma):
            need("patched", ("wop", j), *[("o", r) for r in range(r0, r0 + n, RG)])
            while len(late) >= OUTTOK:
                tok(late.pop(0), new=True)
            ob = pltpu.bitcast(o_ref[r0 // 2:(r0 + n) // 2, :], bf16)
            w = pltpu.bitcast(attach(wop_ref[:, j * 128:(j + 1) * 128], TDO, (NL - 1) * 8, 8, 0), bf16)
            a = jnp.dot(ob, w, preferred_element_type=f32)
            rel.append(a[n - 8:, :])
            res = x_v[r0:r0 + n, j * 128:(j + 1) * 128].astype(f32) * g1_ref[r0:r0 + n, :] + a
            out_v[r0:r0 + n, j * 128:(j + 1) * 128] = res.astype(bf16)
            late.append(res[n - 8:, :])
            done.update(("out", j, r) for r in range(r0, r0 + n, 8))
            if dma is not None:
                c0, m = dma
                need(*[("out", j_, r) for j_ in range(c0, c0 + m) for r in range(r0, r0 + n, 8)])
                c = cp(out_v.at[r0:r0 + n, c0 * 128:(c0 + m) * 128],
                       out_hbm.at[0, r0:r0 + n, c0 * 128:(c0 + m) * 128], sem.at[6])
                c.start(); outs.append(c)

        def uses(e):
            return [(a, e - 4 * (1 - a)) for a in range(2) if 0 <= e - 4 * (1 - a) < WIN]

        def window(name, base):
            need(*[(name, j, r) for j in range(NL) for r in range(max(base - HALO, 0), base + RG, 8)])

        def s1(base):
            window("k", base); need(*[("q", j, base + 8 * a) for j in range(NL) for a in range(2)])
            q = [released(q_ref[:, base + 8 * a:base + 8 * a + 8, :]) for a in range(2)]
            ts = {}
            for e in range(NE):
                off = base + HALO + 8 - DIL * e
                kk = k_ref[:, off:off + 8, :]
                for (a, w) in uses(e):
                    ts[a, w] = jnp.sum(q[a] * kk, axis=0)
            t = jnp.concatenate([ts[a, w] for w in range(WIN) for a in range(2)], axis=0)
            return t, pltpu.roll(t, 64, 1)

        def s2(tr):
            u = tr[0] + tr[1]
            return u, pltpu.roll(u, 32, 1)

        def tree(op, x):
            x = op(x[0:4], x[4:8])
            x = op(x[0:2], x[2:4])
            return op(x[0], x[1])

        def s3(base, ur):
            window("v", base); need(("g", base), ("g", base + 8))
            l = (ur[0] + ur[1]).reshape(WIN, RG, 128)
            if base < DIL * (WIN - 1):
                row = jax.lax.broadcasted_iota(i32, (WIN, RG, 128), 1) + base
                l = jnp.where(row >= DIL * jax.lax.broadcasted_iota(i32, (WIN, RG, 128), 0), l, NEG)
            p = jnp.exp2(l - tree(jnp.maximum, l))
            scl = _recip(tree(jnp.add, p)) * g_ref[base:base + RG, :]
            acc = {}
            for e in range(NE):
                off = base + HALO + 8 - DIL * e
                vv = v_ref[:, off:off + 8, :]
                for (a, w) in uses(e):
                    pr = p[w, 8 * a:8 * a + 8, :] * vv
                    acc[a] = pr if a not in acc else acc[a] + pr
            res = jnp.concatenate([acc[0], acc[1]], axis=1) * scl
            ru = pltpu.bitcast(res, u32)
            ru = ru[:, 0:8, :] | ru[:, 8:16, :]
            for j in range(NL):
                o_ref[base // 2:base // 2 + 8, j * 128:(j + 1) * 128] = pltpu.bitcast(res[j].astype(bf16), u32)
                tok(ru[j], new=True)
            done.add(("o", base))

        T, U = {}, {}

        def attn_step(g):
            if 0 <= g - 2 < NU:
                s3((g - 2) * RG, U.pop(g - 2))
            if 0 <= g - 1 < NU:
                U[g - 1] = s2(T.pop(g - 1))
            if g < NU:
                T[g] = s1(g * RG)

        st = {}

        def fold(v):
            v = pltpu.bitcast(v, u32)
            return functools.reduce(lambda a, b: a | b, [v[r:r + 8, :] for r in range(0, v.shape[0], 8)])

        def rowdot(m, w):
            n = m.shape[0]
            pr = m.astype(f32).reshape(n // 8, 8, D) * w
            return jnp.broadcast_to(jnp.sum(pr, axis=-1, keepdims=True), (n // 8, 8, 128)).reshape(n, 128)

        def gate_route(r0, n):
            assert "patched" not in done and (r0 == 0 or ("g", r0 - 8) in done)
            need(*[("x", r // TM) for r in range(r0, r0 + n, 8)])
            x = x_v[r0:r0 + n, :].astype(f32)
            hh = 0.5 * jnp.tanh(0.5 * rowdot(x, released2(cst["gw"])))
            g_ref[r0:r0 + n, :] = 0.5 + hh
            g1_ref[r0:r0 + n, :] = 0.5 - hh
            tok(fold(hh), new=True)
            rl = rowdot(x, released2(cst["wr"])).astype(bf16).astype(f32)
            for r in range(0, n, 8):
                if r0 + r == 0:
                    st["m"], st["i"] = rl[0:8, :], jnp.zeros((8, 128), i32)
                else:
                    better = rl[r:r + 8, :] > st["m"]
                    st["m"] = jnp.where(better, rl[r:r + 8, :], st["m"])
                    st["i"] = jnp.where(better, r0 + r, st["i"])
                done.add(("g", r0 + r))
            tok(st["m"]); tok(st["i"])

        def finish_route():
            need(("g", S - 8))
            m8, i8 = st["m"], st["i"] + jax.lax.broadcasted_iota(i32, (8, 128), 0)
            m = jnp.max(m8, axis=0, keepdims=True)
            idx = jnp.clip(jnp.min(jnp.min(jnp.where(m8 == m, i8, S), axis=0, keepdims=True)), 0, S - 1)
            t16 = pl.multiple_of((idx // 16) * 16, 16)
            xt = x_v[pl.ds(t16, 16), :].astype(f32)
            row = jax.lax.broadcasted_iota(i32, (16, D), 0) + t16
            xs = jnp.sum(jnp.where(row == idx, xt, 0.0), axis=0, keepdims=True)
            st.update(rs=_sigmoid(m), t16=t16, idx=idx, xs=jnp.broadcast_to(xs, (8, D)))

        def ffn_gate(r0, n):
            hg = rowdot(wg_v[r0:r0 + n, :], released2(st["xs"]))
            sg = hg * _sigmoid(hg)
            h_ref[r0:r0 + n, :] = sg
            tok(fold(sg), new=True)
            done.add(("h", r0))

        def ffn_up_down(r0, n):
            need(("h", r0))
            h = h_ref[r0:r0 + n, :] * rowdot(wu_v[r0:r0 + n, :], released2(st["xs"]))
            c = wd_v[r0:r0 + n, :].astype(f32) * jnp.tile(h, (1, NL))
            for r in range(0, n, 8):
                st["y"] = c[0:8, :] if r0 + r == 0 else st["y"] + c[r:r + 8, :]
            done.add(("y", r0))
            yu = pltpu.bitcast(st["y"], u32)
            tok(functools.reduce(lambda a, b: a | b, [yu[:, j * 128:(j + 1) * 128] for j in range(NL)]), new=True)

        def ffn_finish():
            need(*[("y", r) for r in range(0, F, FG)], *[("xp", r) for r in range(0, S, 8)])
            y = jnp.sum(st["y"], axis=0, keepdims=True) * jnp.tile(st["rs"], (1, NL))
            t16 = st["t16"]
            xt = x_v[pl.ds(t16, 16), :].astype(f32)
            row = jax.lax.broadcasted_iota(i32, (16, D), 0) + t16
            x_v[pl.ds(t16, 16), :] = jnp.where(row == st["idx"], xt + y, xt).astype(bf16)
            done.add("patched")

        def region(mx, vp):
            vp = sorted(vp, key=lambda t: t[0])
            k = 0
            for c, chunk in enumerate(mx):
                while k < len(vp) and vp[k][0] < c + 0.5:
                    vp[k][1](); k += 1
                chunk()
            for _, task in vp[k:]:
                task()
            pending.clear(); rel.clear(); delayq.clear()

        def part(i, p, js=range(NL), rows=TM, k0=0, k1=NL):
            return [P(qkv_chunk, i * TM + r, rows, p, j, k0, k1) for j in js for r in range(0, TM, rows)]

        def spread(fn, r0, r1, step, lo, hi):
            rs = list(range(r0, r1, step))
            return [(lo + (hi - lo) * (t + 1) / len(rs), P(fn, r, step)) for t, r in enumerate(rs)]

        wait(w0a)
        start(grp_c)
        cst["never"] = jnp.abs(wqkv_v[0:8, 0:128].astype(f32)) < 0.0
        for kt in range(KS):
            prep_w(0, kt)
        wait(grp_a); done.add(("x", 0))
        cst["gw"] = jnp.broadcast_to(gw_ref[...].astype(f32).reshape(1, D), (8, D))
        cst["wr"] = jnp.broadcast_to(wr_ref[...].astype(f32).reshape(1, D), (8, D))
        repack_x(0, TM)
        region(part(0, 0, range(4), TM, 0, KS) + part(0, 0, (4,), TM // 4, 0, KS), [])
        wait(grp_a2); done.add(("x", 1))
        start(grp_e)
        repack_x(TM, TM)
        for kt in range(KS, NL):
            prep_w(0, kt)
        mx = (part(1, 0, range(4), TM, 0, KS) + part(0, 0, range(NL), TM, KS, NL)
              + part(1, 0, range(NL), TM, KS, NL) + part(1, 0, (4,), TM // 4, 0, KS))
        region(mx, spread(gate_route, 0, TM, XG, G0, G1))
        wait(grp_b); done.update((("x", 2), ("x", 3)))
        repack_x(2 * TM, TM)
        mx = part(2, 0) + part(3, 0, (0, 1, 2)) + part(3, 0, (3, 4), TM // 2)
        n = len(mx)
        region(mx, spread(gate_route, TM, GBE * TM, XG, 1.0, n - 3) + spread(repack_x, 3 * TM, 4 * TM, 64, 0.0, 3.0))
        wait(grp_c); done.add(("x", 4))
        repack_x(4 * TM, TM)
        for p in (1, 2):
            for kt in range(NL):
                prep_w(p, kt)
        allq = part(4, 0)[:QH] + part(0, 1) + part(0, 2)
        avail = {0: len(allq)}
        allq += part(4, 0)[QH:]
        for i in range(1, 5):
            allq += part(i, 1) + part(i, 2)
            avail[i] = len(allq)
        nc = len(allq) // 4 * 4
        for i in range(5, NB):
            allq += part(i, 0) + part(i, 1) + part(i, 2)
            avail[i] = len(allq)
        upb = TM // RG
        a0 = avail[0] + A0
        vp = [(max(a0 + (nc - CEND - a0) * (g + 1) / UA, avail[g // upb] + 1), P(attn_step, g)) for g in range(UA)]
        vp += spread(gate_route, GBE * TM, 5 * TM, XG, 0.05 * nc, 0.3 * nc)
        region(allq[:nc], vp)
        wait(grp_e); done.update(("x", i) for i in (5, 6, 7))
        repack_x(5 * TM, TM)
        mx = allq[nc:]
        nq = len(mx)
        for i in range(NB - 1):
            mx += [P(out_chunk, i * TM, TM, j, (0, NL) if j == NL - 1 else None) for j in range(NL)]
        nbl = len(mx)
        r7, hm = (NB - 1) * TM, TM // 2
        mx += [P(out_chunk, r7, TM, j, (0, 3) if j == 2 else None) for j in range(3)]
        mx += [P(out_chunk, r7 + h * hm, hm, j, (3, 2) if j == 4 else None) for h in range(2) for j in (3, 4)]
        rest = list(range(UA, NU + 2))
        n1 = int(round(EQ * nq))
        vp = []
        for t, g in enumerate(rest):
            pos = (nq - GAP) * (t + 1) / n1 if t < n1 else nq + (nbl - 0.6 - nq) * (t + 1 - n1) / (len(rest) - n1)
            vp.append((max(pos, avail[min(g, NU - 1) // upb] - nc + 1), P(attn_step, g)))
        f0 = FR0 * nq
        f1 = f0 + 0.4 * (nq - f0)
        vp += spread(gate_route, 5 * TM, S, XG, 0.0, f0 - 1)
        vp += spread(repack_x, 6 * TM, S, 64, 0.0, 8)
        vp += [(f0, finish_route)]
        vp += spread(ffn_gate, 0, F, FG, f0 + 1, f1)
        vp += spread(ffn_up_down, 0, F, FG, f1, nq - FE)
        vp += [(0.1 * nq + 0.8 * nq * (j + 1) / NL, P(prep_wo, j)) for j in range(NL)]
        vp += [(nq - FE + 1, ffn_finish)]
        region(mx, vp)
        wait(outs)

    return kernel


def build(**kw):
    kernel = make(**kw)

    @jax.jit
    def fn(A_x, A_wqkv, A_wo, B_x, B_w_r, B_w_gate, B_w_up, B_w_down, gate_w):
        hbm = pl.BlockSpec(memory_space=pltpu.MemorySpace.HBM)
        vm = pltpu.VMEM
        return pl.pallas_call(
            kernel,
            in_specs=[hbm] * 8,
            out_specs=hbm,
            out_shape=jax.ShapeDtypeStruct((1, S, D), bf16),
            scratch_shapes=[
                vm((S, D), bf16), vm((D, 3 * D), bf16), vm((D, D), bf16),
                vm((F, D), bf16), vm((F, D), bf16), vm((F, D), bf16),
                vm((S, D), bf16), vm((D,), bf16), vm((D,), bf16),
                vm((4 * NL, D, 128), f32), vm((3 * D // 2, D), u32), vm((D // 2, D), u32),
                vm((S // 2, D), u32),
                vm((NL, S, 128), f32), vm((NL, S + HALO, 128), f32), vm((NL, S + HALO, 128), f32),
                vm((S // 2, D), u32),
                vm((S, 128), f32), vm((S, 128), f32), vm((F, 128), f32),
                pltpu.SemaphoreType.DMA((7,)),
            ],
            compiler_params=pltpu.CompilerParams(vmem_limit_bytes=110 * 2**20),
        )(A_x, A_wqkv, A_wo, B_w_r, B_w_gate.T, B_w_up.T, B_w_down, gate_w)
    return fn


_impl = build()


@jax.jit
def pallas_gated_mix__sliding_local_dilated__moe_arch_mod__prompt_kernel(
    A_x: jax.Array,
    A_wqkv: jax.Array,
    A_wo: jax.Array,
    B_x: jax.Array,
    B_w_r: jax.Array,
    B_w_gate: jax.Array,
    B_w_up: jax.Array,
    B_w_down: jax.Array,
    gate_w: jax.Array,
):
    return _impl(A_x, A_wqkv, A_wo, B_x, B_w_r, B_w_gate, B_w_up, B_w_down, gate_w)
```

```python
import functools
import math

import jax
import jax.numpy as jnp
import jax.experimental.pallas as pl
import jax.experimental.pallas.tpu as pltpu

S, D, H, DH, WIN, DIL, F = 2048, 640, 32, 20, 8, 2, 1728
NL = D // 128
HALO = 16
TM = 256
NB = S // TM
RG = 16
NU = S // RG
NE = WIN + 4
f32, bf16, u32, i32 = jnp.float32, jnp.bfloat16, jnp.uint32, jnp.int32
LOG2E = math.log2(math.e)
QSCALE = (DH ** -0.5) * LOG2E
NEG = -1e9 * LOG2E
NT = (((1,), (1,)), ((), ()))


def _recip(s):
    inv = pl.reciprocal(s, approx=True)
    return inv * (2.0 - s * inv)


def _tile(v, a, b):
    v = jnp.concatenate([v] * b, axis=1) if b > 1 else v
    return jnp.concatenate([v] * a, axis=0) if a > 1 else v


def _sigmoid(x):
    return 0.5 * jnp.tanh(0.5 * x) + 0.5


def make(XG=16, FG=16, OUTTOK=2, RELD=6, TD=2, TDO=2, UA=56, CEND=3, EQ=0.87, FR0=0.2, GAP=2, FE=2,
         QH=5, A0=1, KS=3, G0=2.0, G1=12.0, GBE=4):

    def kernel(x_hbm, wqkv_hbm, wo_hbm, wr_hbm, wg_hbm, wu_hbm, wd_hbm, gw_hbm, out_hbm,
               x_v, wqkv_v, wo_v, wg_v, wu_v, wd_v, out_v, wr_ref, gw_ref,
               t_ref, wp_ref, wop_ref, xp_ref, q_ref, k_ref, v_ref, o_ref, g_ref, g1_ref, h_ref,
               sem):
        P = functools.partial
        cp = pltpu.make_async_copy

        def wcopy(r0, r1, p, sm):
            return cp(wqkv_hbm.at[r0:r1, p * D:(p + 1) * D], wqkv_v.at[r0:r1, p * D:(p + 1) * D], sem.at[sm])

        def xcopy(i, sm):
            return cp(x_hbm.at[0, i * TM:(i + 1) * TM, :], x_v.at[i * TM:(i + 1) * TM, :], sem.at[sm])

        w0a = [wcopy(kt * 128, (kt + 1) * 128, 0, 0) for kt in range(KS)]
        grp_a = [xcopy(0, 2), cp(wr_hbm, wr_ref, sem.at[2]), cp(gw_hbm, gw_ref, sem.at[2])]
        grp_a2 = [wcopy(KS * 128, D, 0, 1), xcopy(1, 1)]
        grp_b = [xcopy(i, 3) for i in (2, 3)]
        grp_c = [wcopy(0, D, 1, 4), wcopy(0, D, 2, 4), xcopy(4, 4)]
        grp_e = [xcopy(i, 5) for i in (5, 6, 7)] + [
            cp(a, b, sem.at[5]) for a, b in ((wo_hbm, wo_v), (wg_hbm, wg_v), (wu_hbm, wu_v), (wd_hbm, wd_v))]
        outs = []

        def start(g):
            for c in g:
                c.start()

        def wait(g):
            for c in g:
                c.wait()

        done = set()

        def need(*keys):
            for k_ in keys:
                assert k_ in done, k_

        start(w0a); start(grp_a); start(grp_a2); start(grp_b)
        for j in range(NL):
            k_ref[j, 0:HALO, :] = jnp.zeros((HALO, 128), f32)
            v_ref[j, 0:HALO, :] = jnp.zeros((HALO, 128), f32)

        cst, pending, delayq, rel = {}, [], [], []

        def tok(v, new=False):
            v = v if v.dtype == u32 else pltpu.bitcast(v, u32)
            if pending and not new:
                pending[-1] = pending[-1] | v
            else:
                pending.append(v)

        def attach(a, delay, g0, ng, c0):
            delayq.append(list(pending)); pending.clear()
            toks = delayq.pop(0) if len(delayq) > delay else []
            if not toks:
                return a
            slots = {}
            for n, t in enumerate(toks):
                g = g0 + (n * ng) // len(toks)
                slots[g] = t if g not in slots else slots[g] | t
            rows, prev = [], 0
            for g in sorted(slots):
                if g > prev:
                    rows.append(a[prev * 8:g * 8, :])
                last = jnp.where(cst["never"], slots[g], a[g * 8:(g + 1) * 8, c0 * 128:(c0 + 1) * 128])
                rows.append(jnp.concatenate([a[g * 8:(g + 1) * 8, 0:c0 * 128], last], axis=1) if c0 else last)
                prev = g + 1
            if prev * 8 < a.shape[0]:
                rows.append(a[prev * 8:, :])
            return jnp.concatenate(rows, axis=0)

        def released(v):
            if len(rel) < RELD:
                return v
            r = rel[-RELD] if v.dtype == f32 else pltpu.bitcast(rel[-RELD], v.dtype)
            return jnp.where(cst["never"], r, v)

        def released2(v):
            if len(rel) < RELD:
                return v
            r = rel[-RELD] if v.dtype == f32 else pltpu.bitcast(rel[-RELD], v.dtype)
            reps = (v.shape[0] // 8, v.shape[1] // 128)
            return jnp.where(_tile(cst["never"], *reps), _tile(r, *reps), v)

        def prep_w(p, kt):
            t_ref[p * NL + kt, 0:D, :] = wqkv_v[kt * 128:(kt + 1) * 128, p * D:(p + 1) * D].T.astype(f32)
            for d in range(DH):
                r0 = (p * D + d * H) // 2
                wp_ref[r0:r0 + H // 2, kt * 128:(kt + 1) * 128] = pltpu.bitcast(
                    t_ref[p * NL + kt, pl.ds(d, H, stride=DH), :].astype(bf16), u32)
            done.add(("wp", p, kt))

        def prep_wo(j):
            w = pltpu.bitcast(released2(pltpu.bitcast(wo_v[:, j * 128:(j + 1) * 128], u32)), bf16)
            t_ref[3 * NL + j, 0:D, :] = w.astype(f32)
            for d in range(DH):
                wop_ref[d * H // 2:(d + 1) * H // 2, j * 128:(j + 1) * 128] = pltpu.bitcast(
                    t_ref[3 * NL + j, pl.ds(d, H, stride=DH), :].astype(bf16), u32)
            done.add(("wop", j))

        def repack_x(r0, n):
            assert "patched" not in done
            need(*[("x", r // TM) for r in range(r0, r0 + n, 8)])
            xp_ref[r0 // 2:(r0 + n) // 2, :] = released2(pltpu.bitcast(x_v[r0:r0 + n, :], u32))
            done.update(("xp", r) for r in range(r0, r0 + n, 8))

        def qkv_chunk(r0, n, p, j, k0=0, k1=NL):
            need(*[("xp", r) for r in range(r0, r0 + n, 8)], *[("wp", p, kt) for kt in range(k0, k1)])
            xb = pltpu.bitcast(attach(xp_ref[r0 // 2:(r0 + n) // 2, k0 * 128:k1 * 128], TD, 0, n // 16, k1 - k0 - 1), bf16)
            w0 = (p * D + j * 128) // 2
            r = jax.lax.dot_general(xb, pltpu.bitcast(wp_ref[w0:w0 + 64, k0 * 128:k1 * 128], bf16), NT,
                                    preferred_element_type=f32)
            rel.append(r[n - 8:, :])
            if p == 0:
                first = k1 - k0 < NL and ("qa", j, r0) not in done
                if k1 - k0 < NL and not first:
                    need(*[("qa", j, r_) for r_ in range(r0, r0 + n, 8)])
                    r = r + q_ref[j, r0:r0 + n, :]
                q_ref[j, r0:r0 + n, :] = r if first else r * QSCALE
            else:
                first = False
                (k_ref if p == 1 else v_ref)[j, HALO + r0:HALO + r0 + n, :] = r
            done.update(("qa" if first else "qkv"[p], j, r_) for r_ in range(r0, r0 + n, 8))

        late = []

        def out_chunk(r0, n, j, dma):
            need("patched", ("wop", j), *[("o", r) for r in range(r0, r0 + n, RG)])
            while len(late) >= OUTTOK:
                tok(late.pop(0), new=True)
            ob = pltpu.bitcast(o_ref[r0 // 2:(r0 + n) // 2, :], bf16)
            w = pltpu.bitcast(attach(wop_ref[:, j * 128:(j + 1) * 128], TDO, (NL - 1) * 8, 8, 0), bf16)
            a = jnp.dot(ob, w, preferred_element_type=f32)
            rel.append(a[n - 8:, :])
            res = x_v[r0:r0 + n, j * 128:(j + 1) * 128].astype(f32) * g1_ref[r0:r0 + n, :] + a
            out_v[r0:r0 + n, j * 128:(j + 1) * 128] = res.astype(bf16)
            late.append(res[n - 8:, :])
            done.update(("out", j, r) for r in range(r0, r0 + n, 8))
            if dma is not None:
                c0, m = dma
                need(*[("out", j_, r) for j_ in range(c0, c0 + m) for r in range(r0, r0 + n, 8)])
                c = cp(out_v.at[r0:r0 + n, c0 * 128:(c0 + m) * 128],
                       out_hbm.at[0, r0:r0 + n, c0 * 128:(c0 + m) * 128], sem.at[6])
                c.start(); outs.append(c)

        def uses(e):
            return [(a, e - 4 * (1 - a)) for a in range(2) if 0 <= e - 4 * (1 - a) < WIN]

        def window(name, base):
            need(*[(name, j, r) for j in range(NL) for r in range(max(base - HALO, 0), base + RG, 8)])

        def s1(base):
            window("k", base); need(*[("q", j, base + 8 * a) for j in range(NL) for a in range(2)])
            q = [released(q_ref[:, base + 8 * a:base + 8 * a + 8, :]) for a in range(2)]
            ts = {}
            for e in range(NE):
                off = base + HALO + 8 - DIL * e
                kk = k_ref[:, off:off + 8, :]
                for (a, w) in uses(e):
                    ts[a, w] = jnp.sum(q[a] * kk, axis=0)
            t = jnp.concatenate([ts[a, w] for w in range(WIN) for a in range(2)], axis=0)
            return t, pltpu.roll(t, 64, 1)

        def s2(tr):
            u = tr[0] + tr[1]
            return u, pltpu.roll(u, 32, 1)

        def tree(op, x):
            x = op(x[0:4], x[4:8])
            x = op(x[0:2], x[2:4])
            return op(x[0], x[1])

        def s3(base, ur):
            window("v", base); need(("g", base), ("g", base + 8))
            l = (ur[0] + ur[1]).reshape(WIN, RG, 128)
            if base < DIL * (WIN - 1):
                row = jax.lax.broadcasted_iota(i32, (WIN, RG, 128), 1) + base
                l = jnp.where(row >= DIL * jax.lax.broadcasted_iota(i32, (WIN, RG, 128), 0), l, NEG)
            p = jnp.exp2(l - tree(jnp.maximum, l))
            scl = _recip(tree(jnp.add, p)) * g_ref[base:base + RG, :]
            acc = {}
            for e in range(NE):
                off = base + HALO + 8 - DIL * e
                vv = v_ref[:, off:off + 8, :]
                for (a, w) in uses(e):
                    pr = p[w, 8 * a:8 * a + 8, :] * vv
                    acc[a] = pr if a not in acc else acc[a] + pr
            res = jnp.concatenate([acc[0], acc[1]], axis=1) * scl
            ru = pltpu.bitcast(res, u32)
            ru = ru[:, 0:8, :] | ru[:, 8:16, :]
            for j in range(NL):
                o_ref[base // 2:base // 2 + 8, j * 128:(j + 1) * 128] = pltpu.bitcast(res[j].astype(bf16), u32)
                tok(ru[j], new=True)
            done.add(("o", base))

        T, U = {}, {}

        def attn_step(g):
            if 0 <= g - 2 < NU:
                s3((g - 2) * RG, U.pop(g - 2))
            if 0 <= g - 1 < NU:
                U[g - 1] = s2(T.pop(g - 1))
            if g < NU:
                T[g] = s1(g * RG)

        st = {}

        def fold(v):
            v = pltpu.bitcast(v, u32)
            return functools.reduce(lambda a, b: a | b, [v[r:r + 8, :] for r in range(0, v.shape[0], 8)])

        def rowdot(m, w):
            n = m.shape[0]
            pr = m.astype(f32).reshape(n // 8, 8, D) * w
            return jnp.broadcast_to(jnp.sum(pr, axis=-1, keepdims=True), (n // 8, 8, 128)).reshape(n, 128)

        def gate_route(r0, n):
            assert "patched" not in done and (r0 == 0 or ("g", r0 - 8) in done)
            need(*[("x", r // TM) for r in range(r0, r0 + n, 8)])
            x = x_v[r0:r0 + n, :].astype(f32)
            hh = 0.5 * jnp.tanh(0.5 * rowdot(x, released2(cst["gw"])))
            g_ref[r0:r0 + n, :] = 0.5 + hh
            g1_ref[r0:r0 + n, :] = 0.5 - hh
            tok(fold(hh), new=True)
            rl = rowdot(x, released2(cst["wr"])).astype(bf16).astype(f32)
            for r in range(0, n, 8):
                if r0 + r == 0:
                    st["m"], st["i"] = rl[0:8, :], jnp.zeros((8, 128), i32)
                else:
                    better = rl[r:r + 8, :] > st["m"]
                    st["m"] = jnp.where(better, rl[r:r + 8, :], st["m"])
                    st["i"] = jnp.where(better, r0 + r, st["i"])
                done.add(("g", r0 + r))
            tok(st["m"]); tok(st["i"])

        def finish_route():
            need(("g", S - 8))
            m8, i8 = st["m"], st["i"] + jax.lax.broadcasted_iota(i32, (8, 128), 0)
            m = jnp.max(m8, axis=0, keepdims=True)
            idx = jnp.clip(jnp.min(jnp.min(jnp.where(m8 == m, i8, S), axis=0, keepdims=True)), 0, S - 1)
            t16 = pl.multiple_of((idx // 16) * 16, 16)
            xt = x_v[pl.ds(t16, 16), :].astype(f32)
            row = jax.lax.broadcasted_iota(i32, (16, D), 0) + t16
            xs = jnp.sum(jnp.where(row == idx, xt, 0.0), axis=0, keepdims=True)
            st.update(rs=_sigmoid(m), t16=t16, idx=idx, xs=jnp.broadcast_to(xs, (8, D)))

        def ffn_gate(r0, n):
            hg = rowdot(wg_v[r0:r0 + n, :], released2(st["xs"]))
            sg = hg * _sigmoid(hg)
            h_ref[r0:r0 + n, :] = sg
            tok(fold(sg), new=True)
            done.add(("h", r0))

        def ffn_up_down(r0, n):
            need(("h", r0))
            h = h_ref[r0:r0 + n, :] * rowdot(wu_v[r0:r0 + n, :], released2(st["xs"]))
            c = wd_v[r0:r0 + n, :].astype(f32) * _tile(h, 1, NL)
            for r in range(0, n, 8):
                st["y"] = c[0:8, :] if r0 + r == 0 else st["y"] + c[r:r + 8, :]
            done.add(("y", r0))
            yu = pltpu.bitcast(st["y"], u32)
            tok(functools.reduce(lambda a, b: a | b, [yu[:, j * 128:(j + 1) * 128] for j in range(NL)]), new=True)

        def ffn_finish():
            need(*[("y", r) for r in range(0, F, FG)], *[("xp", r) for r in range(0, S, 8)])
            y = jnp.sum(st["y"], axis=0, keepdims=True) * _tile(st["rs"], 1, NL)
            t16 = st["t16"]
            xt = x_v[pl.ds(t16, 16), :].astype(f32)
            row = jax.lax.broadcasted_iota(i32, (16, D), 0) + t16
            x_v[pl.ds(t16, 16), :] = jnp.where(row == st["idx"], xt + y, xt).astype(bf16)
            done.add("patched")

        def region(mx, vp):
            vp = sorted(vp, key=lambda t: t[0])
            k = 0
            for c, chunk in enumerate(mx):
                while k < len(vp) and vp[k][0] < c + 0.5:
                    vp[k][1](); k += 1
                chunk()
            for _, task in vp[k:]:
                task()
            pending.clear(); rel.clear(); delayq.clear()

        def part(i, p, js=range(NL), rows=TM, k0=0, k1=NL):
            return [P(qkv_chunk, i * TM + r, rows, p, j, k0, k1) for j in js for r in range(0, TM, rows)]

        def spread(fn, r0, r1, step, lo, hi):
            rs = list(range(r0, r1, step))
            return [(lo + (hi - lo) * (t + 1) / len(rs), P(fn, r, step)) for t, r in enumerate(rs)]

        wait(w0a)
        start(grp_c)
        cst["never"] = jnp.abs(wqkv_v[0:8, 0:128].astype(f32)) < 0.0
        for kt in range(KS):
            prep_w(0, kt)
        wait(grp_a); done.add(("x", 0))
        cst["gw"] = jnp.broadcast_to(gw_ref[...].astype(f32).reshape(1, D), (8, D))
        cst["wr"] = jnp.broadcast_to(wr_ref[...].astype(f32).reshape(1, D), (8, D))
        repack_x(0, TM)
        region(part(0, 0, range(4), TM, 0, KS) + part(0, 0, (4,), TM // 4, 0, KS), [])
        wait(grp_a2); done.add(("x", 1))
        start(grp_e)
        repack_x(TM, TM)
        for kt in range(KS, NL):
            prep_w(0, kt)
        mx = (part(1, 0, range(4), TM, 0, KS) + part(0, 0, range(NL), TM, KS, NL)
              + part(1, 0, range(NL), TM, KS, NL) + part(1, 0, (4,), TM // 4, 0, KS))
        region(mx, spread(gate_route, 0, TM, XG, G0, G1))
        wait(grp_b); done.update((("x", 2), ("x", 3)))
        repack_x(2 * TM, TM)
        mx = part(2, 0) + part(3, 0, (0, 1, 2)) + part(3, 0, (3, 4), TM // 2)
        n = len(mx)
        region(mx, spread(gate_route, TM, GBE * TM, XG, 1.0, n - 3) + spread(repack_x, 3 * TM, 4 * TM, 64, 0.0, 3.0))
        wait(grp_c); done.add(("x", 4))
        repack_x(4 * TM, TM)
        for p in (1, 2):
            for kt in range(NL):
                prep_w(p, kt)
        allq = part(4, 0)[:QH] + part(0, 1) + part(0, 2)
        avail = {0: len(allq)}
        allq += part(4, 0)[QH:]
        for i in range(1, 5):
            allq += part(i, 1) + part(i, 2)
            avail[i] = len(allq)
        nc = len(allq) // 4 * 4
        for i in range(5, NB):
            allq += part(i, 0) + part(i, 1) + part(i, 2)
            avail[i] = len(allq)
        upb = TM // RG
        a0 = avail[0] + A0
        vp = [(max(a0 + (nc - CEND - a0) * (g + 1) / UA, avail[g // upb] + 1), P(attn_step, g)) for g in range(UA)]
        vp += spread(gate_route, GBE * TM, 5 * TM, XG, 0.05 * nc, 0.3 * nc)
        region(allq[:nc], vp)
        wait(grp_e); done.update(("x", i) for i in (5, 6, 7))
        repack_x(5 * TM, TM)
        mx = allq[nc:]
        nq = len(mx)
        for i in range(NB - 1):
            mx += [P(out_chunk, i * TM, TM, j, (0, NL) if j == NL - 1 else None) for j in range(NL)]
        nbl = len(mx)
        r7, hm = (NB - 1) * TM, TM // 2
        mx += [P(out_chunk, r7, TM, j, (0, 3) if j == 2 else None) for j in range(3)]
        mx += [P(out_chunk, r7 + h * hm, hm, j, (3, 2) if j == 4 else None) for h in range(2) for j in (3, 4)]
        rest = list(range(UA, NU + 2))
        n1 = int(round(EQ * nq))
        vp = []
        for t, g in enumerate(rest):
            pos = (nq - GAP) * (t + 1) / n1 if t < n1 else nq + (nbl - 0.6 - nq) * (t + 1 - n1) / (len(rest) - n1)
            vp.append((max(pos, avail[min(g, NU - 1) // upb] - nc + 1), P(attn_step, g)))
        f0 = FR0 * nq
        f1 = f0 + 0.4 * (nq - f0)
        vp += spread(gate_route, 5 * TM, S, XG, 0.0, f0 - 1)
        vp += spread(repack_x, 6 * TM, S, 64, 0.0, 8)
        vp += [(f0, finish_route)]
        vp += spread(ffn_gate, 0, F, FG, f0 + 1, f1)
        vp += spread(ffn_up_down, 0, F, FG, f1, nq - FE)
        vp += [(0.1 * nq + 0.8 * nq * (j + 1) / NL, P(prep_wo, j)) for j in range(NL)]
        vp += [(nq - FE + 1, ffn_finish)]
        region(mx, vp)
        wait(outs)

    return kernel


def build(**kw):
    kernel = make(**kw)

    @jax.jit
    def fn(A_x, A_wqkv, A_wo, B_x, B_w_r, B_w_gate, B_w_up, B_w_down, gate_w):
        hbm = pl.BlockSpec(memory_space=pltpu.MemorySpace.HBM)
        vm = pltpu.VMEM
        return pl.pallas_call(
            kernel,
            in_specs=[hbm] * 8,
            out_specs=hbm,
            out_shape=jax.ShapeDtypeStruct((1, S, D), bf16),
            scratch_shapes=[
                vm((S, D), bf16), vm((D, 3 * D), bf16), vm((D, D), bf16),
                vm((F, D), bf16), vm((F, D), bf16), vm((F, D), bf16),
                vm((S, D), bf16), vm((D,), bf16), vm((D,), bf16),
                vm((4 * NL, D + 24, 128), f32), vm((3 * D // 2, D), u32), vm((D // 2, D), u32),
                vm((S // 2, D), u32),
                vm((NL, S, 128), f32), vm((NL, S + HALO, 128), f32), vm((NL, S + HALO, 128), f32),
                vm((S // 2, D), u32),
                vm((S, 128), f32), vm((S, 128), f32), vm((F, 128), f32),
                pltpu.SemaphoreType.DMA((7,)),
            ],
            compiler_params=pltpu.CompilerParams(vmem_limit_bytes=110 * 2**20),
        )(A_x, A_wqkv, A_wo, B_w_r, B_w_gate.T, B_w_up.T, B_w_down, gate_w)
    return fn


_impl = build()


@jax.jit
def pallas_gated_mix__sliding_local_dilated__moe_arch_mod__prompt_kernel(
    A_x: jax.Array,
    A_wqkv: jax.Array,
    A_wo: jax.Array,
    B_x: jax.Array,
    B_w_r: jax.Array,
    B_w_gate: jax.Array,
    B_w_up: jax.Array,
    B_w_down: jax.Array,
    gate_w: jax.Array,
):
    return _impl(A_x, A_wqkv, A_wo, B_x, B_w_r, B_w_gate, B_w_up, B_w_down, gate_w)
```
